```python
import os as _os
_os.environ.setdefault('JAX_PLATFORMS', 'cpu')
import jax
import jax.numpy as jnp

def _softmax(x, axis=-1):
    return jax.nn.softmax(x, axis=axis)

def _gelu(x):
    return jax.nn.gelu(x, approximate=True)

def _silu(x):
    return jax.nn.silu(x)

def _sigmoid(x):
    return jax.nn.sigmoid(x)

def _layernorm(x, axis=-1, eps=1e-05):
    m = jnp.mean(x, axis=axis, keepdims=True)
    v = jnp.var(x, axis=axis, keepdims=True)
    return (x - m) / jnp.sqrt(v + eps)

def _scatter_add(tgt, idx, src, axis=0):
    return tgt.at[idx].add(src)

def _segment_sum(src, seg, n):
    return jax.ops.segment_sum(src, seg, n)

class _Rng:

    def __init__(self, key):
        self._k = key

    def _next(self):
        self._k, sub = jax.random.split(self._k)
        return sub

    def normal(self, shape):
        return jax.random.normal(self._next(), shape, dtype=jnp.bfloat16)

    def randint(self, lo, hi, shape):
        return jax.random.randint(self._next(), shape, lo, hi, dtype=jnp.int32)

    def uniform(self, shape, lo=0.0, hi=1.0):
        return jax.random.uniform(self._next(), shape, jnp.bfloat16, lo, hi)

    def permutation(self, n):
        return jax.random.permutation(self._next(), n)
kernel_name = 'gated_mix__mha_block__memory_aug_recurrent_mem_tr__prompt'

def setup_inputs():
    _rng = _Rng(jax.random.key(int.from_bytes(__import__("os").urandom(4), "little")))
    _w = lambda a: (lambda t: t.astype(jnp.bfloat16) if jnp.issubdtype(t.dtype, jnp.floating) else t)(jnp.asarray(a))

    def _A_setup():
        B, S, D, H = (1, 2048, 512, 32)
        return {'x': _w((lambda *s: _rng.normal(s) * 0.05)(B, S, D)), 'wqkv': _w((lambda *s: _rng.normal(s) * 0.8)(D, 3 * D)), 'wo': _w((lambda *s: _rng.normal(s) * 0.05)(D, D))}
    _A_in = _A_setup()

    def _B_setup():
        B, S, Dm = (1, 2048, 512)
        H, Dh = (32, 128)
        M, seg = (8, 32)
        seg = min(seg, S)
        S = S // seg * seg
        return {'x': _w((lambda *s: _rng.normal(s) * 0.05)(B, S, Dm)), 'mem0': _w((lambda *s: _rng.normal(s) * 0.8)(B, M, Dm)), 'Wq': _w((lambda *s: _rng.normal(s) * 1.6)(Dm, H, Dh) * Dm ** (-0.5)), 'Wk': _w((lambda *s: _rng.normal(s) * 1.6)(Dm, H, Dh) * Dm ** (-0.5)), 'Wv': _w((lambda *s: _rng.normal(s) * 0.8)(Dm, H, Dh) * Dm ** (-0.5)), 'Wo': _w((lambda *s: _rng.normal(s) * 0.8)(H, Dh, Dm) * (H * Dh) ** (-0.5)), 'seg_len': seg}
    _B_in = _B_setup()
    return {'A_x': _A_in['x'], 'A_wqkv': _A_in['wqkv'], 'A_wo': _A_in['wo'], 'B_x': _B_in['x'], 'B_mem0': _B_in['mem0'], 'B_Wq': _B_in['Wq'], 'B_Wk': _B_in['Wk'], 'B_Wv': _B_in['Wv'], 'B_Wo': _B_in['Wo'], 'B_seg_len': _B_in['seg_len'], 'gate_w': _w((lambda *s: _rng.normal(s) * 0.05)(512) * 16.0)}

def reference(A_x, A_wqkv, A_wo, B_x, B_mem0, B_Wq, B_Wk, B_Wv, B_Wo, B_seg_len, gate_w):

    def _A_ref(x, wqkv, wo):
        B, S, D = x.shape
        H = 32
        Dh = D // H
        qkv = (lambda x, *d: x.transpose(*d))((x @ wqkv).reshape(B, S, 3, H, Dh), 2, 0, 3, 1, 4)
        q, k, v = (qkv[0], qkv[1], qkv[2])
        scores = jnp.einsum('bhqd,bhkd->bhqk', q, k) * Dh ** (-0.5)
        p = _softmax(scores, axis=-1)
        o = jnp.einsum('bhqk,bhkd->bhqd', p, v)
        return (lambda x, *d: x.transpose(*d))(o, 0, 2, 1, 3).reshape(B, S, D) @ wo

    def _B_ref(x, mem0, Wq, Wk, Wv, Wo, seg_len):
        B, S, Dm = x.shape
        H, Dh = (Wq.shape[1], Wq.shape[2])
        M = mem0.shape[1]
        scale = Dh ** (-0.5)
        n_seg = S // seg_len
        L = M + seg_len
        idx = jnp.arange(L)
        mask = (idx[:, None] < M) | (idx[:, None] >= idx[None, :])
        mem = mem0
        outs = []
        for s in range(n_seg):
            xs = x[:, s * seg_len:(s + 1) * seg_len, :].copy()
            h = jnp.concatenate([mem, xs], axis=1)
            q = jnp.einsum('btd,dhe->bhte', h, Wq)
            k = jnp.einsum('btd,dhe->bhte', h, Wk)
            v = jnp.einsum('btd,dhe->bhte', h, Wv)
            scores = jnp.einsum('bhqe,bhke->bhqk', q, k) * scale
            scores = jnp.where(mask[None, None], scores, -1000000000.0)
            p = _softmax(scores, axis=-1)
            o = jnp.einsum('bhqk,bhke->bhqe', p, v)
            o = jnp.einsum('bhte,hed->btd', o, Wo)
            mem = o[:, :M, :].copy()
            outs.append(o[:, M:, :])
        return jnp.concatenate(outs, axis=1)
    x = A_x
    g = _sigmoid((x * gate_w).sum(-1, keepdims=True))
    a = _A_ref(x, A_wqkv, A_wo)
    b = _B_ref(x, B_mem0, B_Wq, B_Wk, B_Wv, B_Wo, B_seg_len)
    return g * a + (1 - g) * b
```

```python
import functools
import jax
import jax.numpy as jnp
from jax import lax
import jax.experimental.pallas as pl
import jax.experimental.pallas.tpu as pltpu

BF = jnp.bfloat16
F32 = jnp.float32


def _kernel(x_ref, wqkv_ref, woa_ref, mem0_ref, wq_ref, wk_ref, wv_ref, wob_ref, gw_ref,
            out_ref,
            qT_scr, k_scr, vT_scr, oT_scr, b_scr,
            *, S, D, HA, DHA, M, SEG, HB, DHB, QB):
    x = x_ref[...]

    qkv = jnp.dot(x, wqkv_ref[...], preferred_element_type=F32)
    scale_a = DHA ** -0.5
    q = qkv[:, 0:D] * scale_a
    k = qkv[:, D:2 * D]
    v = qkv[:, 2 * D:3 * D]
    qT_scr[...] = q.T.astype(BF)
    k_scr[...] = k.astype(BF)
    vT_scr[...] = v.T.astype(BF)

    HPG = 128 // DHA
    n_qb = S // QB

    def head_body(h, carry):
        g = h // HPG
        j = h % HPG
        goff = pl.multiple_of(g * 128, 128)
        kg = k_scr[:, pl.ds(goff, 128)]
        qg = qT_scr[pl.ds(goff, 128), :]
        rows = lax.broadcasted_iota(jnp.int32, (128, S), 0)
        qpad = jnp.where((rows // DHA) == j, qg, jnp.zeros_like(qg))
        vT_h = vT_scr[pl.ds(pl.multiple_of(h * DHA, DHA), DHA), :]
        ones_row = (lax.broadcasted_iota(jnp.int32, (DHA, S), 0) == 0).astype(BF)
        vTe = jnp.concatenate([vT_h, ones_row], axis=0)
        for qb in range(n_qb):
            sT = jnp.dot(kg, qpad[:, qb * QB:(qb + 1) * QB], preferred_element_type=F32)
            m = jnp.max(sT, axis=0, keepdims=True)
            pT = jnp.exp(sT - m).astype(BF)
            oe = jnp.dot(vTe, pT, preferred_element_type=F32)
            o = oe[0:DHA, :] / oe[DHA:DHA + 1, :]
            oT_scr[pl.ds(pl.multiple_of(h * DHA, DHA), DHA), qb * QB:(qb + 1) * QB] = o.astype(BF)
        return carry

    lax.fori_loop(0, HA, head_body, 0)

    a = lax.dot_general(oT_scr[...], woa_ref[...], (((0,), (0,)), ((), ())),
                        preferred_element_type=F32)

    L = M + SEG
    n_seg = S // SEG
    scale_b = DHB ** -0.5
    ri = lax.broadcasted_iota(jnp.int32, (L, L), 0)
    ci = lax.broadcasted_iota(jnp.int32, (L, L), 1)
    mask = (ri < M) | (ri >= ci)

    def seg_body(s, mem):
        xs = x_ref[pl.ds(pl.multiple_of(s * SEG, SEG), SEG), :].astype(F32)
        hcat = jnp.concatenate([mem, xs], axis=0).astype(BF)
        qb_ = jnp.dot(hcat, wq_ref[...], preferred_element_type=F32).astype(BF)
        kb_ = jnp.dot(hcat, wk_ref[...], preferred_element_type=F32).astype(BF)
        vb_ = jnp.dot(hcat, wv_ref[...], preferred_element_type=F32).astype(BF)
        outs = []
        for h in range(HB):
            sl = slice(h * DHB, (h + 1) * DHB)
            sc = lax.dot_general(qb_[:, sl], kb_[:, sl], (((1,), (1,)), ((), ())),
                                 preferred_element_type=F32) * scale_b
            sc = jnp.where(mask, sc, -1e9)
            mx = jnp.max(sc, axis=-1, keepdims=True)
            e = jnp.exp(sc - mx)
            p = e / jnp.sum(e, axis=-1, keepdims=True)
            outs.append(jnp.dot(p.astype(BF), vb_[:, sl], preferred_element_type=F32).astype(BF))
        o = jnp.concatenate(outs, axis=1)
        out = jnp.dot(o, wob_ref[...], preferred_element_type=F32)
        b_scr[pl.ds(pl.multiple_of(s * SEG, SEG), SEG), :] = out[M:, :]
        return out[:M, :].astype(BF).astype(F32)

    lax.fori_loop(0, n_seg, seg_body, mem0_ref[...].astype(F32))

    gl = jnp.sum(x.astype(F32) * gw_ref[...].astype(F32), axis=-1, keepdims=True)
    g = jax.nn.sigmoid(gl)
    out_ref[...] = (g * a + (1.0 - g) * b_scr[...]).astype(out_ref.dtype)


@functools.partial(jax.jit, static_argnames=("B_seg_len",))
def pallas_gated_mix__mha_block__memory_aug_recurrent_mem_tr__prompt_kernel(A_x, A_wqkv, A_wo, B_x, B_mem0, B_Wq, B_Wk, B_Wv, B_Wo, B_seg_len, gate_w):
    del B_x
    B, S, D = A_x.shape
    HA = 32
    DHA = D // HA
    Dm, HB, DHB = B_Wq.shape
    M = B_mem0.shape[1]
    SEG = int(B_seg_len)
    x = A_x.reshape(S, D)
    mem0 = B_mem0.reshape(M, Dm)
    wq = B_Wq.reshape(Dm, HB * DHB)
    wk = B_Wk.reshape(Dm, HB * DHB)
    wv = B_Wv.reshape(Dm, HB * DHB)
    wob = B_Wo.reshape(HB * DHB, Dm)
    gw = gate_w.reshape(1, D)
    kern = functools.partial(_kernel, S=S, D=D, HA=HA, DHA=DHA, M=M, SEG=SEG, HB=HB, DHB=DHB, QB=256)
    out = pl.pallas_call(
        kern,
        out_shape=jax.ShapeDtypeStruct((S, D), A_x.dtype),
        scratch_shapes=[
            pltpu.VMEM((D, S), BF), pltpu.VMEM((S, D), BF), pltpu.VMEM((D, S), BF),
            pltpu.VMEM((D, S), BF), pltpu.VMEM((S, D), F32),
        ],
        compiler_params=pltpu.CompilerParams(vmem_limit_bytes=110 * 1024 * 1024),
    )(x, A_wqkv, A_wo, mem0, wq, wk, wv, wob, gw)
    return out.reshape(B, S, D)
```

```python
import functools, os
import jax
import jax.numpy as jnp
from jax import lax
import jax.experimental.pallas as pl
import jax.experimental.pallas.tpu as pltpu

PH = os.environ.get('DEV_PHASES', 'AB')
BF = jnp.bfloat16
F32 = jnp.float32
LOG2E = 1.4426950408889634
NEG = -1e9


def _attn_a(k_scr, qT_scr, vT_scr, oT_scr, sA, sB, mA, mB, qp, *, S, HA, DHA, QB, KC):
    HPG = 128 // DHA
    NQ = S // QB
    U = HA * NQ
    NC = S // KC

    def produce_setup(u):
        h = u // NQ
        qb = u % NQ
        g = h // HPG
        j = h % HPG
        goff = pl.multiple_of(g * 128, 128)
        qoff = pl.multiple_of(qb * QB, QB)
        qg = qT_scr[pl.ds(goff, 128), pl.ds(qoff, QB)]
        rows = lax.broadcasted_iota(jnp.int32, (128, QB), 0)
        qp[...] = jnp.where((rows // DHA) == j, qg, jnp.zeros_like(qg))
        return goff

    def step(up, uc, s_prod, m_prod, s_cons, m_cons, do_cons=True):
        goff = produce_setup(up)
        if do_cons:
            hc = uc // NQ
            qbc = uc % NQ
            hoff = pl.multiple_of(hc * DHA, DHA)
            vT_h = vT_scr[pl.ds(hoff, DHA), :]
            ones_row = (lax.broadcasted_iota(jnp.int32, (DHA, S), 0) == 0).astype(BF)
            vTe = jnp.concatenate([vT_h, ones_row], axis=0)
            mc = m_cons[...]
        mrun = None
        acc = None
        for c in range(NC):
            kc = k_scr[c * KC:(c + 1) * KC, pl.ds(goff, 128)]
            s = jnp.dot(kc, qp[...], preferred_element_type=F32)
            s_prod[c * KC:(c + 1) * KC, :] = s
            cm = jnp.max(s.reshape(KC // 8, 8, QB), axis=0)
            mrun = cm if mrun is None else jnp.maximum(mrun, cm)
            if do_cons:
                sc = s_cons[c * KC:(c + 1) * KC, :]
                p = jnp.exp2(sc - mc).astype(BF)
                d = jnp.dot(vTe[:, c * KC:(c + 1) * KC], p, preferred_element_type=F32)
                acc = d if acc is None else acc + d
        m_prod[...] = jnp.max(mrun, axis=0, keepdims=True)
        if do_cons:
            o = acc[0:DHA, :] / acc[DHA:DHA + 1, :]
            oT_scr[pl.ds(hoff, DHA), pl.ds(pl.multiple_of(qbc * QB, QB), QB)] = o.astype(BF)

    step(0, 0, sA, mA, None, None, do_cons=False)

    def body(i, carry):
        u0 = 2 * i
        step(u0 + 1, u0, sB, mB, sA, mA)
        step(jnp.minimum(u0 + 2, U - 1), u0 + 1, sA, mA, sB, mB)
        return carry

    lax.fori_loop(0, U // 2, body, 0)


def _kernel(x_ref, wqkv_ref, woa_ref, mem0_ref, wq_ref, wk_ref, wv_ref, wob_ref, gw_ref,
            out_ref,
            qT_scr, k_scr, vT_scr, oT_scr, sA, sB, mA, mB, qp,
            wq_p, wk_p, wv_p, wo_p, qpre, kpre, vpre, olate, b_scr,
            *, S, D, HA, DHA, M, SEG, HB, DHB):
    x = x_ref[...]

    qkv = jnp.dot(x, wqkv_ref[...], preferred_element_type=F32)
    q = qkv[:, 0:D] * (DHA ** -0.5 * LOG2E)
    k = qkv[:, D:2 * D]
    v = qkv[:, 2 * D:3 * D]
    qT_scr[...] = q.T.astype(BF)
    k_scr[...] = k.astype(BF)
    vT_scr[...] = v.T.astype(BF)
    if 'A' in PH:
        _attn_a(k_scr, qT_scr, vT_scr, oT_scr, sA, sB, mA, mB, qp,
                S=S, HA=HA, DHA=DHA, QB=512, KC=256)
    a = lax.dot_general(oT_scr[...], woa_ref[...], (((0,), (0,)), ((), ())),
                        preferred_element_type=F32)

    n_seg = S // SEG
    L = M + SEG
    NPRE = n_seg * M
    cq = DHB ** -0.5 * LOG2E

    wq_p[...] = pltpu.bitcast(wq_ref[...], jnp.uint32)
    wk_p[...] = pltpu.bitcast(wk_ref[...], jnp.uint32)
    wv_p[...] = pltpu.bitcast(wv_ref[...], jnp.uint32)
    wo_p[...] = pltpu.bitcast(wob_ref[...], jnp.uint32)

    def wmat(ref):
        return pltpu.bitcast(ref[...], BF)

    x_pre = x.astype(F32).reshape(n_seg, SEG, D)[:, 0:M, :].reshape(NPRE, D).astype(BF)
    qpre[...] = jnp.dot(x_pre, wmat(wq_p), preferred_element_type=F32) * cq
    kpre[...] = jnp.dot(x_pre, wmat(wk_p), preferred_element_type=F32)
    vpre[...] = jnp.dot(x_pre, wmat(wv_p), preferred_element_type=F32)

    ri = lax.broadcasted_iota(jnp.int32, (L, L), 0)
    ci = lax.broadcasted_iota(jnp.int32, (L, L), 1)
    tok_r = jnp.where(ri >= SEG, ri - SEG, ri)
    tok_c = jnp.where(ci >= SEG, ci - SEG, ci)
    mask = (ri < M) | (ci < M) | (tok_r >= tok_c)

    def seg_body(s, mem):
        r0 = pl.multiple_of(s * SEG, SEG)
        p0 = pl.multiple_of(s * M, M)
        xs = x_ref[pl.ds(r0, SEG), :].astype(F32)
        hc = jnp.concatenate([mem, xs[M:SEG, :]], axis=0).astype(BF)
        q_ = jnp.concatenate([jnp.dot(hc, wmat(wq_p), preferred_element_type=F32) * cq,
                              qpre[pl.ds(p0, M), :]], axis=0).astype(BF)
        k_ = jnp.concatenate([jnp.dot(hc, wmat(wk_p), preferred_element_type=F32),
                              kpre[pl.ds(p0, M), :]], axis=0).astype(BF)
        v_ = jnp.concatenate([jnp.dot(hc, wmat(wv_p), preferred_element_type=F32),
                              vpre[pl.ds(p0, M), :]], axis=0).astype(BF)
        outs = []
        for h in range(HB):
            sl = slice(h * DHB, (h + 1) * DHB)
            sc = lax.dot_general(q_[:, sl], k_[:, sl], (((1,), (1,)), ((), ())),
                                 preferred_element_type=F32)
            sc = jnp.where(mask, sc, NEG)
            mx = jnp.max(sc, axis=-1, keepdims=True)
            e = jnp.exp2(sc - mx)
            p = e / jnp.sum(e, axis=-1, keepdims=True)
            outs.append(jnp.dot(p.astype(BF), v_[:, sl], preferred_element_type=F32))
        o = jnp.concatenate(outs, axis=1)
        olate[pl.ds(p0, M), :] = o[SEG:L, :]
        out32 = jnp.dot(o[0:SEG, :].astype(BF), wmat(wo_p), preferred_element_type=F32)
        b_scr[pl.ds(r0 + M, SEG - M), :] = out32[M:SEG, :]
        return out32[0:M, :]

    if 'B' in PH:
        lax.fori_loop(0, n_seg, seg_body, mem0_ref[...].astype(F32))

    res = jnp.dot(olate[...].astype(BF), wmat(wo_p), preferred_element_type=F32)
    for s in range(n_seg):
        b_scr[s * SEG:s * SEG + M, :] = res[s * M:(s + 1) * M, :]

    gl = jnp.sum(x.astype(F32) * gw_ref[...].astype(F32), axis=-1, keepdims=True)
    g = jax.nn.sigmoid(gl)
    out_ref[...] = (g * a + (1.0 - g) * b_scr[...]).astype(out_ref.dtype)


@functools.partial(jax.jit, static_argnames=("B_seg_len",))
def pallas_gated_mix__mha_block__memory_aug_recurrent_mem_tr__prompt_kernel(A_x, A_wqkv, A_wo, B_x, B_mem0, B_Wq, B_Wk, B_Wv, B_Wo, B_seg_len, gate_w):
    del B_x
    B, S, D = A_x.shape
    HA = 32
    DHA = D // HA
    Dm, HB, DHB = B_Wq.shape
    M = B_mem0.shape[1]
    SEG = int(B_seg_len)
    HD = HB * DHB
    n_seg = S // SEG
    x = A_x.reshape(S, D)
    mem0 = B_mem0.reshape(M, Dm)
    wq = B_Wq.reshape(Dm, HD)
    wk = B_Wk.reshape(Dm, HD)
    wv = B_Wv.reshape(Dm, HD)
    wob = B_Wo.reshape(HD, Dm)
    gw = gate_w.reshape(1, D)
    QB = 512
    kern = functools.partial(_kernel, S=S, D=D, HA=HA, DHA=DHA, M=M, SEG=SEG, HB=HB, DHB=DHB)
    out = pl.pallas_call(
        kern,
        out_shape=jax.ShapeDtypeStruct((S, D), A_x.dtype),
        scratch_shapes=[
            pltpu.VMEM((D, S), BF), pltpu.VMEM((S, D), BF), pltpu.VMEM((D, S), BF), pltpu.VMEM((D, S), BF),
            pltpu.VMEM((S, QB), F32), pltpu.VMEM((S, QB), F32),
            pltpu.VMEM((1, QB), F32), pltpu.VMEM((1, QB), F32),
            pltpu.VMEM((128, QB), BF),
            pltpu.VMEM((Dm // 2, HD), jnp.uint32), pltpu.VMEM((Dm // 2, HD), jnp.uint32),
            pltpu.VMEM((Dm // 2, HD), jnp.uint32), pltpu.VMEM((HD // 2, Dm), jnp.uint32),
            pltpu.VMEM((n_seg * M, HD), F32), pltpu.VMEM((n_seg * M, HD), F32), pltpu.VMEM((n_seg * M, HD), F32),
            pltpu.VMEM((n_seg * M, HD), F32),
            pltpu.VMEM((S, D), F32),
        ],
        compiler_params=pltpu.CompilerParams(vmem_limit_bytes=120 * 1024 * 1024),
    )(x, A_wqkv, A_wo, mem0, wq, wk, wv, wob, gw)
    return out.reshape(B, S, D)
```

```python
import functools, os
import jax
import jax.numpy as jnp
from jax import lax
import jax.experimental.pallas as pl
import jax.experimental.pallas.tpu as pltpu

BF = jnp.bfloat16
F32 = jnp.float32
LOG2E = 1.4426950408889634
NEG = -1e9
PGW = int(os.environ.get('PGW', 1024))
WKC = int(os.environ.get('WKC', 4))
PATTERN = os.environ.get('PATTERN', '')


def _make_a(k_scr, qT_scr, vT_scr, oT_scr, sA, sB, mA, mB, qp, *, S, HA, DHA, QB, KC):
    HPG = 128 // DHA
    NQ = S // QB
    U = HA * NQ
    NC = S // KC

    def produce_setup(u):
        h = u // NQ
        qb = u % NQ
        g = h // HPG
        j = h % HPG
        goff = pl.multiple_of(g * 128, 128)
        qoff = pl.multiple_of(qb * QB, QB)
        qg = qT_scr[pl.ds(goff, 128), pl.ds(qoff, QB)]
        rows = lax.broadcasted_iota(jnp.int32, (128, QB), 0)
        qp[...] = jnp.where((rows // DHA) == j, qg, jnp.zeros_like(qg))
        return goff

    def step(up, uc, s_prod, m_prod, s_cons, m_cons, do_cons=True):
        goff = produce_setup(up)
        if do_cons:
            hc = uc // NQ
            qbc = uc % NQ
            hoff = pl.multiple_of(hc * DHA, DHA)
            vT_h = vT_scr[pl.ds(hoff, DHA), :]
            ones_row = (lax.broadcasted_iota(jnp.int32, (DHA, S), 0) == 0).astype(BF)
            vTe = jnp.concatenate([vT_h, ones_row], axis=0)
            mc = m_cons[...]
        mrun = None
        acc = None
        for c in range(NC):
            kc = k_scr[c * KC:(c + 1) * KC, pl.ds(goff, 128)]
            s = jnp.dot(kc, qp[...], preferred_element_type=F32)
            s_prod[c * KC:(c + 1) * KC, :] = s
            cm = jnp.max(s.reshape(KC // 8, 8, QB), axis=0)
            mrun = cm if mrun is None else jnp.maximum(mrun, cm)
            if do_cons:
                sc = s_cons[c * KC:(c + 1) * KC, :]
                p = jnp.exp2(sc - mc).astype(BF)
                d = jnp.dot(vTe[:, c * KC:(c + 1) * KC], p, preferred_element_type=F32)
                acc = d if acc is None else acc + d
            if c < NC - 1:
                yield
        m_prod[...] = jnp.max(mrun, axis=0, keepdims=True)
        if do_cons:
            o = acc[0:DHA, :] / acc[DHA:DHA + 1, :]
            oT_scr[pl.ds(hoff, DHA), pl.ds(pl.multiple_of(qbc * QB, QB), QB)] = o.astype(BF)
        yield

    def prologue():
        for _ in step(0, 0, sA, mA, None, None, do_cons=False):
            pass

    def gen(i):
        u0 = 2 * i
        yield from step(u0 + 1, u0, sB, mB, sA, mA)
        yield from step(jnp.minimum(u0 + 2, U - 1), u0 + 1, sA, mA, sB, mB)

    return prologue, gen, 2 * NC


def _kernel(x_ref, wqkv_ref, woa_ref, mem0_ref, wq_ref, wk_ref, wv_ref, wob_ref, gw_ref,
            out_ref,
            qT_scr, k_scr, vT_scr, oT_scr, sA, sB, mA, mB, qp,
            wq_p, wk_p, wv_p, wo_p, qpre, kpre, vpre, olate, b_scr, maskf,
            wq_raw, wk_raw, wv_raw, wo_raw, t0, t1, sems,
            *, S, D, HA, DHA, M, SEG, HB, DHB):
    copies = [pltpu.make_async_copy(src_, dst_, sems.at[i])
              for i, (src_, dst_) in enumerate(((wq_ref, wq_raw), (wk_ref, wk_raw), (wv_ref, wv_raw), (wob_ref, wo_raw)))]
    for cp in copies:
        cp.start()

    x = x_ref[...]

    qkv = jnp.dot(x, wqkv_ref[...], preferred_element_type=F32)
    q = qkv[:, 0:D] * (DHA ** -0.5 * LOG2E)
    k = qkv[:, D:2 * D]
    v = qkv[:, 2 * D:3 * D]
    qT_scr[...] = q.T.astype(BF)
    k_scr[...] = k.astype(BF)
    vT_scr[...] = v.T.astype(BF)
    a_prologue, a_gen, n_a = _make_a(k_scr, qT_scr, vT_scr, oT_scr, sA, sB, mA, mB, qp,
                                     S=S, HA=HA, DHA=DHA, QB=512, KC=256)

    n_seg = S // SEG
    L = M + SEG
    NPRE = n_seg * M
    HD = HB * DHB
    cq = DHB ** -0.5 * LOG2E

    def wcols(ref, lo, hi):
        return pltpu.bitcast(ref[:, lo:hi], BF)

    def wrows(ref, lo, hi):
        return pltpu.bitcast(ref[lo // 2:hi // 2, :], BF)

    for cp in copies:
        cp.wait()

    HP = HB // 2
    Dm = D
    RP = Dm * HB // 2 // HP

    def step1_piece(raw, t, i):
        t[i * RP:(i + 1) * RP, :] = pltpu.bitcast(raw[2 * i * RP:2 * (i + 1) * RP, :], jnp.uint32)

    def unit(t, dst, hp):
        ev = t[pl.ds(hp, Dm // 2, stride=2 * HP), :]
        od = t[pl.ds(HP + hp, Dm // 2, stride=2 * HP), :]
        dst[:, (2 * hp) * DHB:(2 * hp + 1) * DHB] = (ev & jnp.uint32(0xFFFF)) | (od << 16)
        dst[:, (2 * hp + 1) * DHB:(2 * hp + 2) * DHB] = (ev >> 16) | (od & jnp.uint32(0xFFFF0000))

    x_pre = x.astype(F32).reshape(n_seg, SEG, D)[:, 0:M, :].reshape(NPRE, D).astype(BF)

    def prepass(w_p, pre, scl, hp):
        lo, hi = 2 * hp * DHB, (2 * hp + 2) * DHB
        y = jnp.dot(x_pre, wcols(w_p, lo, hi), preferred_element_type=F32)
        if scl is not None:
            y = y * scl
        pre[:, lo:hi] = y.astype(BF)

    WOP = HD // 2 // HP

    def wo_piece(i):
        wo_p[i * WOP:(i + 1) * WOP, :] = pltpu.bitcast(wo_raw[2 * i * WOP:2 * (i + 1) * WOP, :], jnp.uint32)

    for i in range(HP):
        step1_piece(wq_raw, t0, i)
    plan = ((wq_raw, t0, wq_p, qpre, cq), (wk_raw, t1, wk_p, kpre, None), (wv_raw, t0, wv_p, vpre, None))
    prev = None
    for mi, (raw, t, w_p, pre, scl) in enumerate(plan):
        for hp in range(HP):
            unit(t, w_p, hp)
            if mi + 1 < len(plan):
                step1_piece(plan[mi + 1][0], plan[mi + 1][1], hp)
            else:
                wo_piece(hp)
            if prev is not None:
                prepass(*prev)
            prev = (w_p, pre, scl, hp)
    prepass(*prev)

    ri = lax.broadcasted_iota(jnp.int32, (L, L), 0)
    ci = lax.broadcasted_iota(jnp.int32, (L, L), 1)
    tok_r = jnp.where(ri >= SEG, ri - SEG, ri)
    tok_c = jnp.where(ci >= SEG, ci - SEG, ci)
    mask = (ri < M) | (ci < M) | (tok_r >= tok_c)
    maskf[...] = jnp.concatenate([mask.astype(F32)] * HB, axis=0)

    a_prologue()

    NG = HD // PGW
    HPGp = PGW // DHB

    def b_gen(s, mem, res):
        r0 = pl.multiple_of(s * SEG, SEG)
        p0 = pl.multiple_of(s * M, M)
        xs = x_ref[pl.ds(r0, SEG), :].astype(F32)
        hc = jnp.concatenate([mem, xs[M:SEG, :]], axis=0).astype(BF)
        qs, ks, vs = [], [], []
        for w_p, pre, lst, sc_ in ((wq_p, qpre, qs, cq), (wk_p, kpre, ks, None), (wv_p, vpre, vs, None)):
            for g in range(NG):
                lo, hi = g * PGW, (g + 1) * PGW
                y = jnp.dot(hc, wcols(w_p, lo, hi), preferred_element_type=F32)
                if sc_ is not None:
                    y = y * sc_
                lst.append(jnp.concatenate([y.astype(BF), pre[pl.ds(p0, M), lo:hi]], axis=0))
                yield

        def head(lst, h):
            g, hh = divmod(h, HPGp)
            return lst[g][:, hh * DHB:(hh + 1) * DHB]

        scs = []
        for h in range(HB):
            scs.append(lax.dot_general(head(qs, h), head(ks, h), (((1,), (1,)), ((), ())),
                                       preferred_element_type=F32))
            if h % 8 == 7:
                yield
        sc = jnp.concatenate(scs, axis=0)
        sc = jnp.where(maskf[...] > 0.5, sc, NEG)
        mx = jnp.max(sc, axis=-1, keepdims=True)
        e = jnp.exp2(sc - mx)
        p = e * (1.0 / jnp.sum(e, axis=-1, keepdims=True))
        yield
        HPW = HB // WKC
        out32 = None
        lates = []
        for kc in range(WKC):
            outs = []
            for h in range(kc * HPW, (kc + 1) * HPW):
                outs.append(jnp.dot(p[h * L:(h + 1) * L, :].astype(BF), head(vs, h), preferred_element_type=F32))
            o = jnp.concatenate(outs, axis=1)
            lates.append(o[SEG:L, :])
            yield
            d = jnp.dot(o[0:SEG, :].astype(BF), wrows(wo_p, kc * HPW * DHB, (kc + 1) * HPW * DHB),
                        preferred_element_type=F32)
            out32 = d if out32 is None else out32 + d
            yield
        olate[pl.ds(p0, M), :] = jnp.concatenate(lates, axis=1).astype(BF)
        b_scr[pl.ds(r0 + M, SEG - M), :] = out32[M:SEG, :]
        res.append(out32[0:M, :])

    def merged_body(s, mem):
        res = []
        gb = b_gen(s, mem, res)
        ga = a_gen(s)
        a_done = b_done = False
        while not (a_done and b_done):
            if not b_done:
                try:
                    next(gb)
                except StopIteration:
                    b_done = True
            if not a_done:
                try:
                    next(ga)
                except StopIteration:
                    a_done = True
        return res[0]

    lax.fori_loop(0, n_seg, merged_body, mem0_ref[...].astype(F32))

    a = lax.dot_general(oT_scr[...], woa_ref[...], (((0,), (0,)), ((), ())),
                        preferred_element_type=F32)
    res = jnp.dot(olate[...], wrows(wo_p, 0, HD), preferred_element_type=F32)
    for s in range(n_seg):
        b_scr[s * SEG:s * SEG + M, :] = res[s * M:(s + 1) * M, :]

    gl = jnp.sum(x.astype(F32) * gw_ref[...].astype(F32), axis=-1, keepdims=True)
    g = jax.nn.sigmoid(gl)
    out_ref[...] = (g * a + (1.0 - g) * b_scr[...]).astype(out_ref.dtype)


@functools.partial(jax.jit, static_argnames=("B_seg_len",))
def pallas_gated_mix__mha_block__memory_aug_recurrent_mem_tr__prompt_kernel(A_x, A_wqkv, A_wo, B_x, B_mem0, B_Wq, B_Wk, B_Wv, B_Wo, B_seg_len, gate_w):
    del B_x
    B, S, D = A_x.shape
    HA = 32
    DHA = D // HA
    Dm, HB, DHB = B_Wq.shape
    M = B_mem0.shape[1]
    SEG = int(B_seg_len)
    HD = HB * DHB
    n_seg = S // SEG
    x = A_x.reshape(S, D)
    mem0 = B_mem0.reshape(M, Dm)
    wq = B_Wq.reshape(Dm * HB, DHB)
    wk = B_Wk.reshape(Dm * HB, DHB)
    wv = B_Wv.reshape(Dm * HB, DHB)
    wob = B_Wo.reshape(HD, Dm)
    gw = gate_w.reshape(1, D)
    QB = 512
    kern = functools.partial(_kernel, S=S, D=D, HA=HA, DHA=DHA, M=M, SEG=SEG, HB=HB, DHB=DHB)
    out = pl.pallas_call(
        kern,
        out_shape=jax.ShapeDtypeStruct((S, D), A_x.dtype),
        scratch_shapes=[
            pltpu.VMEM((D, S), BF), pltpu.VMEM((S, D), BF), pltpu.VMEM((D, S), BF), pltpu.VMEM((D, S), BF),
            pltpu.VMEM((S, QB), F32), pltpu.VMEM((S, QB), F32),
            pltpu.VMEM((1, QB), F32), pltpu.VMEM((1, QB), F32),
            pltpu.VMEM((128, QB), BF),
            pltpu.VMEM((Dm // 2, HD), jnp.uint32), pltpu.VMEM((Dm // 2, HD), jnp.uint32),
            pltpu.VMEM((Dm // 2, HD), jnp.uint32), pltpu.VMEM((HD // 2, Dm), jnp.uint32),
            pltpu.VMEM((n_seg * M, HD), BF), pltpu.VMEM((n_seg * M, HD), BF), pltpu.VMEM((n_seg * M, HD), BF),
            pltpu.VMEM((n_seg * M, HD), BF),
            pltpu.VMEM((S, D), F32),
            pltpu.VMEM((HB * (M + SEG), M + SEG), F32),
            pltpu.VMEM((Dm * HB, DHB), BF), pltpu.VMEM((Dm * HB, DHB), BF), pltpu.VMEM((Dm * HB, DHB), BF),
            pltpu.VMEM((HD, Dm), BF),
            pltpu.VMEM((Dm * HB // 2, DHB), jnp.uint32), pltpu.VMEM((Dm * HB // 2, DHB), jnp.uint32),
            pltpu.SemaphoreType.DMA((4,)),
        ],
        in_specs=[
            pl.BlockSpec(memory_space=pltpu.VMEM), pl.BlockSpec(memory_space=pltpu.VMEM),
            pl.BlockSpec(memory_space=pltpu.VMEM), pl.BlockSpec(memory_space=pltpu.VMEM),
            pl.BlockSpec(memory_space=pl.ANY), pl.BlockSpec(memory_space=pl.ANY),
            pl.BlockSpec(memory_space=pl.ANY), pl.BlockSpec(memory_space=pl.ANY),
            pl.BlockSpec(memory_space=pltpu.VMEM),
        ],
        out_specs=pl.BlockSpec(memory_space=pltpu.VMEM),
        compiler_params=pltpu.CompilerParams(vmem_limit_bytes=120 * 1024 * 1024),
    )(x, A_wqkv, A_wo, mem0, wq, wk, wv, wob, gw)
    return out.reshape(B, S, D)
```

```python
import functools

import jax
import jax.numpy as jnp
from jax import lax
import jax.experimental.pallas as pl
import jax.experimental.pallas.tpu as pltpu

BF = jnp.bfloat16
F32 = jnp.float32
U32 = jnp.uint32
LOG2E = 1.4426950408889634
NEG_INF_SCORE = -1e9

A_QB = 512
A_KC = 256
B_PGW = 1024
B_WKC = 2
UNROLL = 2
T_PAD = 32


def _branch_a(k_scr, qT_scr, vT_scr, oT_scr, sA, sB, mA, mB, qp, *, S, HA, DHA, QB, KC):
    HPG = 128 // DHA
    NQ = S // QB
    U = HA * NQ
    NC = S // KC

    def produce_setup(u):
        h = u // NQ
        qb = u % NQ
        g = h // HPG
        j = h % HPG
        goff = pl.multiple_of(g * 128, 128)
        qoff = pl.multiple_of(qb * QB, QB)
        qg = qT_scr[pl.ds(goff, 128), pl.ds(qoff, QB)]
        rows = lax.broadcasted_iota(jnp.int32, (128, QB), 0)
        qp[...] = pltpu.bitcast(jnp.where((rows // DHA) == j, qg, jnp.zeros_like(qg)), U32)
        return goff

    def step(up, uc, s_prod, m_prod, s_cons, m_cons):
        do_cons = s_cons is not None
        goff = produce_setup(up)
        if do_cons:
            hoff = pl.multiple_of((uc // NQ) * DHA, DHA)
            qoff = pl.multiple_of((uc % NQ) * QB, QB)
            ones_row = (lax.broadcasted_iota(jnp.int32, (DHA, S), 0) == 0).astype(BF)
            vTe = jnp.concatenate([vT_scr[pl.ds(hoff, DHA), :], ones_row], axis=0)
            mc = m_cons[...]
        mrun = None
        acc = None
        for c in range(NC):
            kc = pltpu.bitcast(k_scr[c * KC // 2:(c + 1) * KC // 2, pl.ds(goff, 128)], BF)
            s = jnp.dot(kc, pltpu.bitcast(qp[...], BF), preferred_element_type=F32)
            s_prod[c * KC:(c + 1) * KC, :] = s
            cm = jnp.max(s.reshape(KC // 8, 8, QB), axis=0)
            mrun = cm if mrun is None else jnp.maximum(mrun, cm)
            if do_cons:
                p = jnp.exp2(s_cons[c * KC:(c + 1) * KC, :] - mc).astype(BF)
                d = jnp.dot(vTe[:, c * KC:(c + 1) * KC], p, preferred_element_type=F32)
                acc = d if acc is None else acc + d
            if c < NC - 1:
                yield
        m_prod[...] = jnp.max(mrun, axis=0, keepdims=True)
        if do_cons:
            o = acc[0:DHA, :] / acc[DHA:DHA + 1, :]
            oT_scr[pl.ds(hoff, DHA), pl.ds(qoff, QB)] = o.astype(BF)
        yield

    def prologue():
        for _ in step(0, None, sA, mA, None, None):
            pass

    def gen(i):
        u0 = 2 * i
        yield from step(u0 + 1, u0, sB, mB, sA, mA)
        yield from step(jnp.minimum(u0 + 2, U - 1), u0 + 1, sA, mA, sB, mB)

    return prologue, gen


def _kernel(x_ref, wqkv_ref, woa_ref, mem0_ref, wq_hbm, wk_hbm, wv_hbm, wob_hbm, gw_ref,
            out_ref,
            qT_scr, k_scr, vT_scr, oT_scr, sA, sB, mA, mB, qp,
            wq_p, wk_p, wv_p, wo_p, qpre, kpre, vpre, olate, b_scr, maskf,
            wq_raw, wk_raw, wv_raw, wo_raw, t0, t1, sems,
            *, S, D, HA, DHA, M, SEG, HB, DHB):
    copies = [pltpu.make_async_copy(src, dst, sems.at[i]) for i, (src, dst) in enumerate(
        ((wq_hbm, wq_raw), (wk_hbm, wk_raw), (wv_hbm, wv_raw), (wob_hbm, wo_raw)))]
    for cp in copies:
        cp.start()

    x = x_ref[...]

    qkv = jnp.dot(x, wqkv_ref[...], preferred_element_type=F32)
    qT_scr[...] = (qkv[:, 0:D] * (DHA ** -0.5 * LOG2E)).T.astype(BF)
    k_scr[...] = pltpu.bitcast(qkv[:, D:2 * D].astype(BF), U32)
    vT_scr[...] = qkv[:, 2 * D:3 * D].T.astype(BF)
    a_prologue, a_gen = _branch_a(k_scr, qT_scr, vT_scr, oT_scr, sA, sB, mA, mB, qp,
                                  S=S, HA=HA, DHA=DHA, QB=A_QB, KC=A_KC)

    n_seg = S // SEG
    L = M + SEG
    NPRE = n_seg * M
    HD = HB * DHB
    HP = HB // 2
    cq = DHB ** -0.5 * LOG2E

    def wcols(ref, lo, hi):
        return pltpu.bitcast(ref[:, lo:hi], BF)

    def wrows(ref, lo, hi):
        return pltpu.bitcast(ref[lo // 2:hi // 2, :], BF)

    for cp in copies:
        cp.wait()

    RP = D * HB // 2 // HP

    def step1_piece(raw, t, i):
        t[i * RP:(i + 1) * RP, :] = pltpu.bitcast(raw[2 * i * RP:2 * (i + 1) * RP, :], U32)

    def unit(t, dst, hp):
        ev = t[pl.ds(hp, D // 2, stride=2 * HP), :]
        od = t[pl.ds(HP + hp, D // 2, stride=2 * HP), :]
        dst[:, (2 * hp) * DHB:(2 * hp + 1) * DHB] = (ev & jnp.uint32(0xFFFF)) | (od << 16)
        dst[:, (2 * hp + 1) * DHB:(2 * hp + 2) * DHB] = (ev >> 16) | (od & jnp.uint32(0xFFFF0000))

    WOP = HD // 2 // HP

    def wo_piece(i):
        wo_p[i * WOP:(i + 1) * WOP, :] = pltpu.bitcast(wo_raw[2 * i * WOP:2 * (i + 1) * WOP, :], U32)

    x_pre = x.astype(F32).reshape(n_seg, SEG, D)[:, 0:M, :].reshape(NPRE, D).astype(BF)

    def prepass(w_p, pre, scl, hp):
        lo, hi = 2 * hp * DHB, (2 * hp + 2) * DHB
        y = jnp.dot(x_pre, wcols(w_p, lo, hi), preferred_element_type=F32)
        if scl is not None:
            y = y * scl
        pre[:, lo:hi] = y.astype(BF)

    for i in range(HP):
        step1_piece(wq_raw, t0, i)
    plan = ((wq_raw, t0, wq_p, qpre, cq), (wk_raw, t1, wk_p, kpre, None), (wv_raw, t0, wv_p, vpre, None))
    prev = None
    for mi, (raw, t, w_p, pre, scl) in enumerate(plan):
        for hp in range(HP):
            unit(t, w_p, hp)
            if mi + 1 < len(plan):
                step1_piece(plan[mi + 1][0], plan[mi + 1][1], hp)
            else:
                wo_piece(hp)
            if prev is not None:
                prepass(*prev)
            prev = (w_p, pre, scl, hp)
    prepass(*prev)

    ri = lax.broadcasted_iota(jnp.int32, (L, L), 0)
    ci = lax.broadcasted_iota(jnp.int32, (L, L), 1)
    tok_r = jnp.where(ri >= SEG, ri - SEG, ri)
    tok_c = jnp.where(ci >= SEG, ci - SEG, ci)
    mask = (ri < M) | (ci < M) | (tok_r >= tok_c)
    maskf[...] = jnp.concatenate([mask.astype(F32)] * HB, axis=0)

    a_prologue()

    NG = HD // B_PGW
    HPG = B_PGW // DHB
    HPW = HB // B_WKC

    def b_gen(s, mem, res):
        r0 = pl.multiple_of(s * SEG, SEG)
        p0 = pl.multiple_of(s * M, M)
        xs = x_ref[pl.ds(r0, SEG), :].astype(F32)
        hc = jnp.concatenate([mem, xs[M:SEG, :]], axis=0).astype(BF)
        qs, ks, vs = [], [], []
        for w_p, pre, lst, scl in ((wq_p, qpre, qs, cq), (wk_p, kpre, ks, None), (wv_p, vpre, vs, None)):
            for g in range(NG):
                lo, hi = g * B_PGW, (g + 1) * B_PGW
                y = jnp.dot(hc, wcols(w_p, lo, hi), preferred_element_type=F32)
                if scl is not None:
                    y = y * scl
                lst.append(jnp.concatenate([y.astype(BF), pre[pl.ds(p0, M), lo:hi]], axis=0))
                yield

        def head(lst, h):
            g, hh = divmod(h, HPG)
            return lst[g][:, hh * DHB:(hh + 1) * DHB]

        scs = []
        for h in range(HB):
            scs.append(lax.dot_general(head(qs, h), head(ks, h), (((1,), (1,)), ((), ())),
                                       preferred_element_type=F32))
            if h % 8 == 7:
                yield
        sc = jnp.concatenate(scs, axis=0)
        sc = jnp.where(maskf[...] > 0.5, sc, NEG_INF_SCORE * LOG2E)
        e = jnp.exp2(sc - jnp.max(sc, axis=-1, keepdims=True))
        p = e * (1.0 / jnp.sum(e, axis=-1, keepdims=True))
        yield
        out32 = None
        lates = []
        for kc in range(B_WKC):
            outs = [jnp.dot(p[h * L:(h + 1) * L, :].astype(BF), head(vs, h), preferred_element_type=F32)
                    for h in range(kc * HPW, (kc + 1) * HPW)]
            o = jnp.concatenate(outs, axis=1)
            lates.append(o[SEG:L, :])
            yield
            d = jnp.dot(o[0:SEG, :].astype(BF), wrows(wo_p, kc * HPW * DHB, (kc + 1) * HPW * DHB),
                        preferred_element_type=F32)
            out32 = d if out32 is None else out32 + d
            yield
        olate[pl.ds(p0, M), :] = jnp.concatenate(lates, axis=1).astype(BF)
        b_scr[pl.ds(r0 + M, SEG - M), :] = out32[M:SEG, :]
        res.append(out32[0:M, :])

    def merged_body(s, mem):
        res = []
        ga, gb = a_gen(s), b_gen(s, mem, res)
        a_live = b_live = True
        while a_live or b_live:
            if a_live:
                a_live = next(ga, 'done') != 'done'
            if b_live:
                b_live = next(gb, 'done') != 'done'
        return res[0]

    lax.fori_loop(0, n_seg, merged_body, mem0_ref[...].astype(F32), unroll=UNROLL)

    a = lax.dot_general(oT_scr[...], woa_ref[...], (((0,), (0,)), ((), ())),
                        preferred_element_type=F32)
    res = jnp.dot(olate[...], wrows(wo_p, 0, HD), preferred_element_type=F32)
    for s in range(n_seg):
        b_scr[s * SEG:s * SEG + M, :] = res[s * M:(s + 1) * M, :]

    gl = jnp.sum(x.astype(F32) * gw_ref[...].astype(F32), axis=-1, keepdims=True)
    g = jax.nn.sigmoid(gl)
    out_ref[...] = (g * a + (1.0 - g) * b_scr[...]).astype(out_ref.dtype)


@functools.partial(jax.jit, static_argnames=("B_seg_len",))
def pallas_gated_mix__mha_block__memory_aug_recurrent_mem_tr__prompt_kernel(A_x, A_wqkv, A_wo, B_x, B_mem0, B_Wq, B_Wk, B_Wv, B_Wo, B_seg_len, gate_w):
    del B_x
    B, S, D = A_x.shape
    HA = 32
    DHA = D // HA
    Dm, HB, DHB = B_Wq.shape
    M = B_mem0.shape[1]
    SEG = int(B_seg_len)
    HD = HB * DHB
    n_seg = S // SEG
    assert B == 1 and Dm == D and S % SEG == 0 and S % A_QB == 0 and S % A_KC == 0
    assert 128 % DHA == 0 and DHA % 16 == 0 and DHB == 128 and HB % 2 == 0
    assert M % 8 == 0 and SEG % 16 == 0 and M < SEG and HD % B_PGW == 0 and HB % B_WKC == 0
    assert (HA * (S // A_QB)) % 2 == 0 and HA * (S // A_QB) // 2 == n_seg and n_seg % UNROLL == 0
    vmem = pl.BlockSpec(memory_space=pltpu.VMEM)
    hbm = pl.BlockSpec(memory_space=pl.ANY)
    kern = functools.partial(_kernel, S=S, D=D, HA=HA, DHA=DHA, M=M, SEG=SEG, HB=HB, DHB=DHB)
    out = pl.pallas_call(
        kern,
        out_shape=jax.ShapeDtypeStruct((S, D), A_x.dtype),
        in_specs=[vmem, vmem, vmem, vmem, hbm, hbm, hbm, hbm, vmem],
        out_specs=vmem,
        scratch_shapes=[
            pltpu.VMEM((D, S), BF),
            pltpu.VMEM((S // 2, D), U32),
            pltpu.VMEM((D, S), BF),
            pltpu.VMEM((D, S), BF),
            pltpu.VMEM((S, A_QB), F32),
            pltpu.VMEM((S, A_QB), F32),
            pltpu.VMEM((1, A_QB), F32),
            pltpu.VMEM((1, A_QB), F32),
            pltpu.VMEM((64, A_QB), U32),
            pltpu.VMEM((D // 2, HD), U32),
            pltpu.VMEM((D // 2, HD), U32),
            pltpu.VMEM((D // 2, HD), U32),
            pltpu.VMEM((HD // 2, D), U32),
            pltpu.VMEM((n_seg * M, HD), BF),
            pltpu.VMEM((n_seg * M, HD), BF),
            pltpu.VMEM((n_seg * M, HD), BF),
            pltpu.VMEM((n_seg * M, HD), BF),
            pltpu.VMEM((S, D), F32),
            pltpu.VMEM((HB * (M + SEG), M + SEG), F32),
            pltpu.VMEM((D * HB, DHB), BF),
            pltpu.VMEM((D * HB, DHB), BF),
            pltpu.VMEM((D * HB, DHB), BF),
            pltpu.VMEM((HD, D), BF),
            pltpu.VMEM((D * HB // 2 + T_PAD, DHB), U32),
            pltpu.VMEM((D * HB // 2 + T_PAD, DHB), U32),
            pltpu.SemaphoreType.DMA((4,)),
        ],
        compiler_params=pltpu.CompilerParams(vmem_limit_bytes=120 * 1024 * 1024),
    )(A_x.reshape(S, D), A_wqkv, A_wo, B_mem0.reshape(M, D),
      B_Wq.reshape(D * HB, DHB), B_Wk.reshape(D * HB, DHB), B_Wv.reshape(D * HB, DHB),
      B_Wo.reshape(HD, D), gate_w.reshape(1, D))
    return out.reshape(B, S, D)
```

```python
import functools

import jax
import jax.numpy as jnp
from jax import lax
import jax.experimental.pallas as pl
import jax.experimental.pallas.tpu as pltpu

BF = jnp.bfloat16
F32 = jnp.float32
U32 = jnp.uint32
LOG2E = 1.4426950408889634
NEG_INF_SCORE = -1e9

A_QB = 512
A_KC = 256
B_PGW = 1024
B_WKC = 2
UNROLL = 2
X_CH = 512
T_PAD = 32


def _branch_a(k_scr, qT_scr, vT_scr, oT_scr, sA, sB, mA, mB, qp, *, S, HA, DHA, QB, KC):
    HPG = 128 // DHA
    NQ = S // QB
    U = HA * NQ
    NC = S // KC

    def produce_setup(u):
        h = u // NQ
        qb = u % NQ
        g = h // HPG
        j = h % HPG
        goff = pl.multiple_of(g * 128, 128)
        qoff = pl.multiple_of(qb * QB, QB)
        qg = qT_scr[pl.ds(goff, 128), pl.ds(qoff, QB)]
        rows = lax.broadcasted_iota(jnp.int32, (128, QB), 0)
        qp[...] = pltpu.bitcast(jnp.where((rows // DHA) == j, qg, jnp.zeros_like(qg)), U32)
        return goff

    def step(up, uc, s_prod, m_prod, s_cons, m_cons):
        do_cons = s_cons is not None
        goff = produce_setup(up)
        if do_cons:
            hoff = pl.multiple_of((uc // NQ) * DHA, DHA)
            qoff = pl.multiple_of((uc % NQ) * QB, QB)
            ones_row = (lax.broadcasted_iota(jnp.int32, (DHA, S), 0) == 0).astype(BF)
            vTe = jnp.concatenate([vT_scr[pl.ds(hoff, DHA), :], ones_row], axis=0)
            mc = m_cons[...]
        mrun = None
        acc = None
        for c in range(NC):
            kc = pltpu.bitcast(k_scr[c * KC // 2:(c + 1) * KC // 2, pl.ds(goff, 128)], BF)
            s = jnp.dot(kc, pltpu.bitcast(qp[...], BF), preferred_element_type=F32)
            s_prod[c * KC:(c + 1) * KC, :] = s
            cm = jnp.max(s.reshape(KC // 8, 8, QB), axis=0)
            mrun = cm if mrun is None else jnp.maximum(mrun, cm)
            if do_cons:
                p = jnp.exp2(s_cons[c * KC:(c + 1) * KC, :] - mc).astype(BF)
                d = jnp.dot(vTe[:, c * KC:(c + 1) * KC], p, preferred_element_type=F32)
                acc = d if acc is None else acc + d
            if c < NC - 1:
                yield
        m_prod[...] = jnp.max(mrun, axis=0, keepdims=True)
        if do_cons:
            o = acc[0:DHA, :] / acc[DHA:DHA + 1, :]
            oT_scr[pl.ds(hoff, DHA), pl.ds(qoff, QB)] = o.astype(BF)
        yield

    def prologue():
        for _ in step(0, None, sA, mA, None, None):
            pass

    def gen(i):
        u0 = 2 * i
        yield from step(u0 + 1, u0, sB, mB, sA, mA)
        yield from step(jnp.minimum(u0 + 2, U - 1), u0 + 1, sA, mA, sB, mB)

    return prologue, gen


def _kernel(x_hbm, wqkv_hbm, woa_hbm, mem0_ref, wq_hbm, wk_hbm, wv_hbm, wob_hbm, gw_ref,
            out_hbm,
            x_ref, wqkv_ref, woa_ref, out_ref, osems,
            qT_scr, k_scr, vT_scr, oT_scr, sA, sB, mA, mB, qp,
            wq_p, wk_p, wv_p, wo_p, qpre, kpre, vpre, olate, b_scr, maskf,
            wq_raw, wk_raw, wv_raw, wo_raw, t0, t1, sems,
            *, S, D, HA, DHA, M, SEG, HB, DHB):
    NXC = S // X_CH
    x_copies = [pltpu.make_async_copy(x_hbm.at[pl.ds(c * X_CH, X_CH), :], x_ref.at[pl.ds(c * X_CH, X_CH), :],
                                      sems.at[c]) for c in range(NXC)]
    wqkv_copy = pltpu.make_async_copy(wqkv_hbm, wqkv_ref, sems.at[NXC])
    copies = [pltpu.make_async_copy(src, dst, sems.at[NXC + 1 + i]) for i, (src, dst) in enumerate(
        ((wq_hbm, wq_raw), (wk_hbm, wk_raw), (wv_hbm, wv_raw), (wob_hbm, wo_raw), (woa_hbm, woa_ref)))]
    wqkv_copy.start()
    for cp in x_copies + copies:
        cp.start()

    wqkv_copy.wait()
    for c in range(NXC):
        x_copies[c].wait()
        qkv = jnp.dot(x_ref[c * X_CH:(c + 1) * X_CH, :], wqkv_ref[...], preferred_element_type=F32)
        qT_scr[:, c * X_CH:(c + 1) * X_CH] = (qkv[:, 0:D] * (DHA ** -0.5 * LOG2E)).T.astype(BF)
        k_scr[c * X_CH // 2:(c + 1) * X_CH // 2, :] = pltpu.bitcast(qkv[:, D:2 * D].astype(BF), U32)
        vT_scr[:, c * X_CH:(c + 1) * X_CH] = qkv[:, 2 * D:3 * D].T.astype(BF)
    a_prologue, a_gen = _branch_a(k_scr, qT_scr, vT_scr, oT_scr, sA, sB, mA, mB, qp,
                                  S=S, HA=HA, DHA=DHA, QB=A_QB, KC=A_KC)

    n_seg = S // SEG
    L = M + SEG
    NPRE = n_seg * M
    HD = HB * DHB
    HP = HB // 2
    cq = DHB ** -0.5 * LOG2E

    def wcols(ref, lo, hi):
        return pltpu.bitcast(ref[:, lo:hi], BF)

    def wrows(ref, lo, hi):
        return pltpu.bitcast(ref[lo // 2:hi // 2, :], BF)

    copies[0].wait()

    RP = D * HB // 2 // HP

    def step1_piece(raw, t, i):
        t[i * RP:(i + 1) * RP, :] = pltpu.bitcast(raw[2 * i * RP:2 * (i + 1) * RP, :], U32)

    def unit(t, dst, hp):
        ev = t[pl.ds(hp, D // 2, stride=2 * HP), :]
        od = t[pl.ds(HP + hp, D // 2, stride=2 * HP), :]
        dst[:, (2 * hp) * DHB:(2 * hp + 1) * DHB] = (ev & jnp.uint32(0xFFFF)) | (od << 16)
        dst[:, (2 * hp + 1) * DHB:(2 * hp + 2) * DHB] = (ev >> 16) | (od & jnp.uint32(0xFFFF0000))

    WOP = HD // 2 // HP

    def wo_piece(i):
        wo_p[i * WOP:(i + 1) * WOP, :] = pltpu.bitcast(wo_raw[2 * i * WOP:2 * (i + 1) * WOP, :], U32)

    x_pre = x_ref[...].astype(F32).reshape(n_seg, SEG, D)[:, 0:M, :].reshape(NPRE, D).astype(BF)

    def prepass(w_p, pre, scl, hp):
        lo, hi = 2 * hp * DHB, (2 * hp + 2) * DHB
        y = jnp.dot(x_pre, wcols(w_p, lo, hi), preferred_element_type=F32)
        if scl is not None:
            y = y * scl
        pre[:, lo:hi] = y.astype(BF)

    for i in range(HP):
        step1_piece(wq_raw, t0, i)
    plan = ((wq_raw, t0, wq_p, qpre, cq), (wk_raw, t1, wk_p, kpre, None), (wv_raw, t0, wv_p, vpre, None))
    prev = None
    for mi, (raw, t, w_p, pre, scl) in enumerate(plan):
        copies[mi + 1].wait()
        for hp in range(HP):
            unit(t, w_p, hp)
            if mi + 1 < len(plan):
                step1_piece(plan[mi + 1][0], plan[mi + 1][1], hp)
            else:
                wo_piece(hp)
            if prev is not None:
                prepass(*prev)
            prev = (w_p, pre, scl, hp)
    prepass(*prev)

    ri = lax.broadcasted_iota(jnp.int32, (L, L), 0)
    ci = lax.broadcasted_iota(jnp.int32, (L, L), 1)
    tok_r = jnp.where(ri >= SEG, ri - SEG, ri)
    tok_c = jnp.where(ci >= SEG, ci - SEG, ci)
    mask = (ri < M) | (ci < M) | (tok_r >= tok_c)
    maskf[...] = jnp.concatenate([mask.astype(F32)] * HB, axis=0)

    a_prologue()

    NG = HD // B_PGW
    HPG = B_PGW // DHB
    HPW = HB // B_WKC

    def b_gen(s, mem, res):
        r0 = pl.multiple_of(s * SEG, SEG)
        p0 = pl.multiple_of(s * M, M)
        xs = x_ref[pl.ds(r0, SEG), :].astype(F32)
        hc = jnp.concatenate([mem, xs[M:SEG, :]], axis=0).astype(BF)
        qs, ks, vs = [], [], []
        for w_p, pre, lst, scl in ((wq_p, qpre, qs, cq), (wk_p, kpre, ks, None), (wv_p, vpre, vs, None)):
            for g in range(NG):
                lo, hi = g * B_PGW, (g + 1) * B_PGW
                y = jnp.dot(hc, wcols(w_p, lo, hi), preferred_element_type=F32)
                if scl is not None:
                    y = y * scl
                lst.append(jnp.concatenate([y.astype(BF), pre[pl.ds(p0, M), lo:hi]], axis=0))
                yield

        def head(lst, h):
            g, hh = divmod(h, HPG)
            return lst[g][:, hh * DHB:(hh + 1) * DHB]

        scs = []
        for h in range(HB):
            scs.append(lax.dot_general(head(qs, h), head(ks, h), (((1,), (1,)), ((), ())),
                                       preferred_element_type=F32))
            if h % 8 == 7:
                yield
        sc = jnp.concatenate(scs, axis=0)
        sc = jnp.where(maskf[...] > 0.5, sc, NEG_INF_SCORE * LOG2E)
        e = jnp.exp2(sc - jnp.max(sc, axis=-1, keepdims=True))
        p = e * (1.0 / jnp.sum(e, axis=-1, keepdims=True))
        yield
        out32 = None
        lates = []
        for kc in range(B_WKC):
            outs = [jnp.dot(p[h * L:(h + 1) * L, :].astype(BF), head(vs, h), preferred_element_type=F32)
                    for h in range(kc * HPW, (kc + 1) * HPW)]
            o = jnp.concatenate(outs, axis=1)
            lates.append(o[SEG:L, :])
            yield
            d = jnp.dot(o[0:SEG, :].astype(BF), wrows(wo_p, kc * HPW * DHB, (kc + 1) * HPW * DHB),
                        preferred_element_type=F32)
            out32 = d if out32 is None else out32 + d
            yield
        olate[pl.ds(p0, M), :] = jnp.concatenate(lates, axis=1).astype(BF)
        b_scr[pl.ds(r0 + M, SEG - M), :] = out32[M:SEG, :]
        res.append(out32[0:M, :])

    def merged_body(s, mem):
        res = []
        ga, gb = a_gen(s), b_gen(s, mem, res)
        a_live = b_live = True
        while a_live or b_live:
            if a_live:
                a_live = next(ga, 'done') != 'done'
            if b_live:
                b_live = next(gb, 'done') != 'done'
        return res[0]

    lax.fori_loop(0, n_seg, merged_body, mem0_ref[...].astype(F32), unroll=UNROLL)

    copies[4].wait()
    SPC = X_CH // SEG
    out_copies = []
    for c in range(NXC):
        lo, hi = c * X_CH, (c + 1) * X_CH
        a = lax.dot_general(oT_scr[:, lo:hi], woa_ref[...], (((0,), (0,)), ((), ())),
                            preferred_element_type=F32)
        res = jnp.dot(olate[c * SPC * M:(c + 1) * SPC * M, :], wrows(wo_p, 0, HD),
                      preferred_element_type=F32)
        for s in range(SPC):
            b_scr[lo + s * SEG:lo + s * SEG + M, :] = res[s * M:(s + 1) * M, :]
        gl = jnp.sum(x_ref[lo:hi, :].astype(F32) * gw_ref[...].astype(F32), axis=-1, keepdims=True)
        g = jax.nn.sigmoid(gl)
        out_ref[lo:hi, :] = (g * a + (1.0 - g) * b_scr[lo:hi, :]).astype(out_ref.dtype)
        cp = pltpu.make_async_copy(out_ref.at[pl.ds(lo, X_CH), :], out_hbm.at[pl.ds(lo, X_CH), :], osems.at[c])
        cp.start()
        out_copies.append(cp)
    for cp in out_copies:
        cp.wait()


@functools.partial(jax.jit, static_argnames=("B_seg_len",))
def pallas_gated_mix__mha_block__memory_aug_recurrent_mem_tr__prompt_kernel(A_x, A_wqkv, A_wo, B_x, B_mem0, B_Wq, B_Wk, B_Wv, B_Wo, B_seg_len, gate_w):
    del B_x
    B, S, D = A_x.shape
    HA = 32
    DHA = D // HA
    Dm, HB, DHB = B_Wq.shape
    M = B_mem0.shape[1]
    SEG = int(B_seg_len)
    HD = HB * DHB
    n_seg = S // SEG
    assert S % X_CH == 0 and X_CH % SEG == 0
    assert B == 1 and Dm == D and S % SEG == 0 and S % A_QB == 0 and S % A_KC == 0
    assert 128 % DHA == 0 and DHA % 16 == 0 and DHB == 128 and HB % 2 == 0
    assert M % 8 == 0 and SEG % 16 == 0 and M < SEG and HD % B_PGW == 0 and HB % B_WKC == 0
    assert (HA * (S // A_QB)) % 2 == 0 and HA * (S // A_QB) // 2 == n_seg and n_seg % UNROLL == 0
    vmem = pl.BlockSpec(memory_space=pltpu.VMEM)
    hbm = pl.BlockSpec(memory_space=pl.ANY)
    kern = functools.partial(_kernel, S=S, D=D, HA=HA, DHA=DHA, M=M, SEG=SEG, HB=HB, DHB=DHB)
    out = pl.pallas_call(
        kern,
        out_shape=jax.ShapeDtypeStruct((S, D), A_x.dtype),
        in_specs=[hbm, hbm, hbm, vmem, hbm, hbm, hbm, hbm, vmem],
        out_specs=hbm,
        scratch_shapes=[
            pltpu.VMEM((S, D), BF),
            pltpu.VMEM((D, 3 * D), BF),
            pltpu.VMEM((D, D), BF),
            pltpu.VMEM((S, D), A_x.dtype),
            pltpu.SemaphoreType.DMA((S // X_CH,)),
            pltpu.VMEM((D, S), BF),
            pltpu.VMEM((S // 2, D), U32),
            pltpu.VMEM((D, S), BF),
            pltpu.VMEM((D, S), BF),
            pltpu.VMEM((S, A_QB), F32),
            pltpu.VMEM((S, A_QB), F32),
            pltpu.VMEM((1, A_QB), F32),
            pltpu.VMEM((1, A_QB), F32),
            pltpu.VMEM((64, A_QB), U32),
            pltpu.VMEM((D // 2, HD), U32),
            pltpu.VMEM((D // 2, HD), U32),
            pltpu.VMEM((D // 2, HD), U32),
            pltpu.VMEM((HD // 2, D), U32),
            pltpu.VMEM((n_seg * M, HD), BF),
            pltpu.VMEM((n_seg * M, HD), BF),
            pltpu.VMEM((n_seg * M, HD), BF),
            pltpu.VMEM((n_seg * M, HD), BF),
            pltpu.VMEM((S, D), F32),
            pltpu.VMEM((HB * (M + SEG), M + SEG), F32),
            pltpu.VMEM((D * HB, DHB), BF),
            pltpu.VMEM((D * HB, DHB), BF),
            pltpu.VMEM((D * HB, DHB), BF),
            pltpu.VMEM((HD, D), BF),
            pltpu.VMEM((D * HB // 2 + T_PAD, DHB), U32),
            pltpu.VMEM((D * HB // 2 + T_PAD, DHB), U32),
            pltpu.SemaphoreType.DMA((S // X_CH + 6,)),
        ],
        compiler_params=pltpu.CompilerParams(vmem_limit_bytes=120 * 1024 * 1024),
    )(A_x.reshape(S, D), A_wqkv, A_wo, B_mem0.reshape(M, D),
      B_Wq.reshape(D * HB, DHB), B_Wk.reshape(D * HB, DHB), B_Wv.reshape(D * HB, DHB),
      B_Wo.reshape(HD, D), gate_w.reshape(1, D))
    return out.reshape(B, S, D)
```

```python
import functools

import jax
import jax.numpy as jnp
from jax import lax
import jax.experimental.pallas as pl
import jax.experimental.pallas.tpu as pltpu

BF = jnp.bfloat16
F32 = jnp.float32
U32 = jnp.uint32
LOG2E = 1.4426950408889634
NEG_INF_SCORE = -1e9

A_QB = 512
A_KC = 256
B_PGW = 1024
B_WKC = 2
UNROLL = 2
X_CH = 512


def _branch_a(k_scr, qT_scr, vT_scr, oT_scr, sA, sB, mA, mB, qp, *, S, HA, DHA, QB, KC):
    HPG = 128 // DHA
    NQ = S // QB
    U = HA * NQ
    NC = S // KC

    def produce_setup(u):
        h = u // NQ
        qb = u % NQ
        g = h // HPG
        j = h % HPG
        goff = pl.multiple_of(g * 128, 128)
        qoff = pl.multiple_of(qb * QB, QB)
        qg = qT_scr[pl.ds(goff, 128), pl.ds(qoff, QB)]
        rows = lax.broadcasted_iota(jnp.int32, (128, QB), 0)
        qp[...] = pltpu.bitcast(jnp.where((rows // DHA) == j, qg, jnp.zeros_like(qg)), U32)
        return goff

    def step(up, uc, s_prod, m_prod, s_cons, m_cons):
        do_cons = s_cons is not None
        goff = produce_setup(up)
        if do_cons:
            hoff = pl.multiple_of((uc // NQ) * DHA, DHA)
            qoff = pl.multiple_of((uc % NQ) * QB, QB)
            ones_row = (lax.broadcasted_iota(jnp.int32, (DHA, S), 0) == 0).astype(BF)
            vTe = jnp.concatenate([vT_scr[pl.ds(hoff, DHA), :], ones_row], axis=0)
            mc = m_cons[...]
        mrun = None
        acc = None
        for c in range(NC):
            kc = pltpu.bitcast(k_scr[c * KC // 2:(c + 1) * KC // 2, pl.ds(goff, 128)], BF)
            s = jnp.dot(kc, pltpu.bitcast(qp[...], BF), preferred_element_type=F32)
            s_prod[c * KC:(c + 1) * KC, :] = s
            cm = jnp.max(s.reshape(KC // 8, 8, QB), axis=0)
            mrun = cm if mrun is None else jnp.maximum(mrun, cm)
            if do_cons:
                p = jnp.exp2(s_cons[c * KC:(c + 1) * KC, :] - mc).astype(BF)
                d = jnp.dot(vTe[:, c * KC:(c + 1) * KC], p, preferred_element_type=F32)
                acc = d if acc is None else acc + d
            if c < NC - 1:
                yield
        m_prod[...] = jnp.max(mrun, axis=0, keepdims=True)
        if do_cons:
            o = acc[0:DHA, :] / acc[DHA:DHA + 1, :]
            oT_scr[pl.ds(hoff, DHA), pl.ds(qoff, QB)] = o.astype(BF)
        yield

    def prologue():
        for _ in step(0, None, sA, mA, None, None):
            pass

    def gen(i):
        u0 = 2 * i
        yield from step(u0 + 1, u0, sB, mB, sA, mA)
        yield from step(jnp.minimum(u0 + 2, U - 1), u0 + 1, sA, mA, sB, mB)

    return prologue, gen


def _kernel(x_hbm, wqkv_hbm, woa_hbm, mem0_ref, wq_hbm, wk_hbm, wv_hbm, wob_hbm, gw_ref,
            out_hbm,
            x_ref, wqkv_ref, woa_ref, out_ref, osems,
            qT_scr, k_scr, vT_scr, oT_scr, sA, sB, mA, mB, qp,
            wq_p, wk_p, wv_p, wo_p, qpre, kpre, vpre, olate, b_scr, maskf,
            wq_raw, wk_raw, wv_raw, wo_raw, t0, t1, sems,
            *, S, D, HA, DHA, M, SEG, HB, DHB):
    NXC = S // X_CH
    x_copies = [pltpu.make_async_copy(x_hbm.at[pl.ds(c * X_CH, X_CH), :], x_ref.at[pl.ds(c * X_CH, X_CH), :],
                                      sems.at[c]) for c in range(NXC)]
    wqkv_copy = pltpu.make_async_copy(wqkv_hbm, wqkv_ref, sems.at[NXC])
    copies = [pltpu.make_async_copy(src, dst, sems.at[NXC + 1 + i]) for i, (src, dst) in enumerate(
        ((wq_hbm, wq_raw), (wk_hbm, wk_raw), (wv_hbm, wv_raw), (wob_hbm, wo_raw), (woa_hbm, woa_ref)))]
    wqkv_copy.start()
    for cp in x_copies + copies:
        cp.start()

    wqkv_copy.wait()
    for c in range(NXC):
        x_copies[c].wait()
        qkv = jnp.dot(x_ref[c * X_CH:(c + 1) * X_CH, :], wqkv_ref[...], preferred_element_type=F32)
        qT_scr[:, c * X_CH:(c + 1) * X_CH] = (qkv[:, 0:D] * (DHA ** -0.5 * LOG2E)).T.astype(BF)
        k_scr[c * X_CH // 2:(c + 1) * X_CH // 2, :] = pltpu.bitcast(qkv[:, D:2 * D].astype(BF), U32)
        vT_scr[:, c * X_CH:(c + 1) * X_CH] = qkv[:, 2 * D:3 * D].T.astype(BF)
    a_prologue, a_gen = _branch_a(k_scr, qT_scr, vT_scr, oT_scr, sA, sB, mA, mB, qp,
                                  S=S, HA=HA, DHA=DHA, QB=A_QB, KC=A_KC)

    n_seg = S // SEG
    L = M + SEG
    NPRE = n_seg * M
    HD = HB * DHB
    HP = HB // 2
    cq = DHB ** -0.5 * LOG2E

    def wcols(ref, lo, hi):
        return pltpu.bitcast(ref[:, lo:hi], BF)

    def wrows(ref, lo, hi):
        return pltpu.bitcast(ref[lo // 2:hi // 2, :], BF)

    copies[0].wait()

    RP = D * HB // 2 // HP

    def step1_piece(raw, t, i):
        v = pltpu.bitcast(raw[2 * i * RP:2 * (i + 1) * RP, :], U32)
        t[i * RP // HB:(i + 1) * RP // HB, :, :] = v.reshape(RP // HB, HB, DHB)

    def unit(t, dst, hp):
        ev = t[:, hp, :]
        od = t[:, HP + hp, :]
        dst[:, (2 * hp) * DHB:(2 * hp + 1) * DHB] = (ev & jnp.uint32(0xFFFF)) | (od << 16)
        dst[:, (2 * hp + 1) * DHB:(2 * hp + 2) * DHB] = (ev >> 16) | (od & jnp.uint32(0xFFFF0000))

    WOP = HD // 2 // HP

    def wo_piece(i):
        wo_p[i * WOP:(i + 1) * WOP, :] = pltpu.bitcast(wo_raw[2 * i * WOP:2 * (i + 1) * WOP, :], U32)

    x_pre = x_ref[...].astype(F32).reshape(n_seg, SEG, D)[:, 0:M, :].reshape(NPRE, D).astype(BF)

    def prepass(w_p, pre, scl, hp):
        lo, hi = 2 * hp * DHB, (2 * hp + 2) * DHB
        y = jnp.dot(x_pre, wcols(w_p, lo, hi), preferred_element_type=F32)
        if scl is not None:
            y = y * scl
        pre[:, lo:hi] = y.astype(BF)

    for i in range(HP):
        step1_piece(wq_raw, t0, i)
    plan = ((wq_raw, t0, wq_p, qpre, cq), (wk_raw, t1, wk_p, kpre, None), (wv_raw, t0, wv_p, vpre, None))
    prev = None
    for mi, (raw, t, w_p, pre, scl) in enumerate(plan):
        copies[mi + 1].wait()
        for hp in range(HP):
            unit(t, w_p, hp)
            if mi + 1 < len(plan):
                step1_piece(plan[mi + 1][0], plan[mi + 1][1], hp)
            else:
                wo_piece(hp)
            if prev is not None:
                prepass(*prev)
            prev = (w_p, pre, scl, hp)
    prepass(*prev)

    ri = lax.broadcasted_iota(jnp.int32, (L, L), 0)
    ci = lax.broadcasted_iota(jnp.int32, (L, L), 1)
    tok_r = jnp.where(ri >= SEG, ri - SEG, ri)
    tok_c = jnp.where(ci >= SEG, ci - SEG, ci)
    mask = (ri < M) | (ci < M) | (tok_r >= tok_c)
    maskf[...] = jnp.concatenate([mask.astype(F32)] * HB, axis=0)

    a_prologue()

    NG = HD // B_PGW
    HPG = B_PGW // DHB
    HPW = HB // B_WKC

    def b_gen(s, mem, res):
        r0 = pl.multiple_of(s * SEG, SEG)
        p0 = pl.multiple_of(s * M, M)
        xs = x_ref[pl.ds(r0, SEG), :].astype(F32)
        hc = jnp.concatenate([mem, xs[M:SEG, :]], axis=0).astype(BF)
        qs, ks, vs = [], [], []
        for w_p, pre, lst, scl in ((wq_p, qpre, qs, cq), (wk_p, kpre, ks, None), (wv_p, vpre, vs, None)):
            for g in range(NG):
                lo, hi = g * B_PGW, (g + 1) * B_PGW
                y = jnp.dot(hc, wcols(w_p, lo, hi), preferred_element_type=F32)
                if scl is not None:
                    y = y * scl
                lst.append(jnp.concatenate([y.astype(BF), pre[pl.ds(p0, M), lo:hi]], axis=0))
                yield

        def head(lst, h):
            g, hh = divmod(h, HPG)
            return lst[g][:, hh * DHB:(hh + 1) * DHB]

        scs = []
        for h in range(HB):
            scs.append(lax.dot_general(head(qs, h), head(ks, h), (((1,), (1,)), ((), ())),
                                       preferred_element_type=F32))
            if h % 8 == 7:
                yield
        sc = jnp.concatenate(scs, axis=0)
        sc = jnp.where(maskf[...] > 0.5, sc, NEG_INF_SCORE * LOG2E)
        e = jnp.exp2(sc - jnp.max(sc, axis=-1, keepdims=True))
        l = jnp.sum(e, axis=-1, keepdims=True)
        r = pl.reciprocal(l, approx=True)
        p = e * (r * (2.0 - l * r))
        yield
        out32 = None
        lates = []
        for kc in range(B_WKC):
            outs = [jnp.dot(p[h * L:(h + 1) * L, :].astype(BF), head(vs, h), preferred_element_type=F32)
                    for h in range(kc * HPW, (kc + 1) * HPW)]
            o = jnp.concatenate(outs, axis=1)
            lates.append(o[SEG:L, :])
            yield
            d = jnp.dot(o[0:SEG, :].astype(BF), wrows(wo_p, kc * HPW * DHB, (kc + 1) * HPW * DHB),
                        preferred_element_type=F32)
            out32 = d if out32 is None else out32 + d
            yield
        olate[pl.ds(p0, M), :] = jnp.concatenate(lates, axis=1).astype(BF)
        b_scr[pl.ds(r0 + M, SEG - M), :] = out32[M:SEG, :]
        res.append(out32[0:M, :])

    def merged_body(s, mem):
        res = []
        ga, gb = a_gen(s), b_gen(s, mem, res)
        a_live = b_live = True
        while a_live or b_live:
            if a_live:
                a_live = next(ga, 'done') != 'done'
            if b_live:
                b_live = next(gb, 'done') != 'done'
        return res[0]

    lax.fori_loop(0, n_seg, merged_body, mem0_ref[...].astype(F32), unroll=UNROLL)

    copies[4].wait()
    SPC = X_CH // SEG
    out_copies = []
    for c in range(NXC):
        lo, hi = c * X_CH, (c + 1) * X_CH
        a = lax.dot_general(oT_scr[:, lo:hi], woa_ref[...], (((0,), (0,)), ((), ())),
                            preferred_element_type=F32)
        res = jnp.dot(olate[c * SPC * M:(c + 1) * SPC * M, :], wrows(wo_p, 0, HD),
                      preferred_element_type=F32)
        for s in range(SPC):
            b_scr[lo + s * SEG:lo + s * SEG + M, :] = res[s * M:(s + 1) * M, :]
        gl = jnp.sum(x_ref[lo:hi, :].astype(F32) * gw_ref[...].astype(F32), axis=-1, keepdims=True)
        g = jax.nn.sigmoid(gl)
        out_ref[lo:hi, :] = (g * a + (1.0 - g) * b_scr[lo:hi, :]).astype(out_ref.dtype)
        cp = pltpu.make_async_copy(out_ref.at[pl.ds(lo, X_CH), :], out_hbm.at[pl.ds(lo, X_CH), :], osems.at[c])
        cp.start()
        out_copies.append(cp)
    for cp in out_copies:
        cp.wait()


@functools.partial(jax.jit, static_argnames=("B_seg_len",))
def pallas_gated_mix__mha_block__memory_aug_recurrent_mem_tr__prompt_kernel(A_x, A_wqkv, A_wo, B_x, B_mem0, B_Wq, B_Wk, B_Wv, B_Wo, B_seg_len, gate_w):
    del B_x
    B, S, D = A_x.shape
    HA = 32
    DHA = D // HA
    Dm, HB, DHB = B_Wq.shape
    M = B_mem0.shape[1]
    SEG = int(B_seg_len)
    HD = HB * DHB
    n_seg = S // SEG
    assert S % X_CH == 0 and X_CH % SEG == 0
    assert B == 1 and Dm == D and S % SEG == 0 and S % A_QB == 0 and S % A_KC == 0
    assert 128 % DHA == 0 and DHA % 16 == 0 and DHB == 128 and HB % 2 == 0
    assert M % 8 == 0 and SEG % 16 == 0 and M < SEG and HD % B_PGW == 0 and HB % B_WKC == 0
    assert (HA * (S // A_QB)) % 2 == 0 and HA * (S // A_QB) // 2 == n_seg and n_seg % UNROLL == 0
    vmem = pl.BlockSpec(memory_space=pltpu.VMEM)
    hbm = pl.BlockSpec(memory_space=pl.ANY)
    kern = functools.partial(_kernel, S=S, D=D, HA=HA, DHA=DHA, M=M, SEG=SEG, HB=HB, DHB=DHB)
    out = pl.pallas_call(
        kern,
        out_shape=jax.ShapeDtypeStruct((S, D), A_x.dtype),
        in_specs=[hbm, hbm, hbm, vmem, hbm, hbm, hbm, hbm, vmem],
        out_specs=hbm,
        scratch_shapes=[
            pltpu.VMEM((S, D), BF),
            pltpu.VMEM((D, 3 * D), BF),
            pltpu.VMEM((D, D), BF),
            pltpu.VMEM((S, D), A_x.dtype),
            pltpu.SemaphoreType.DMA((S // X_CH,)),
            pltpu.VMEM((D, S), BF),
            pltpu.VMEM((S // 2, D), U32),
            pltpu.VMEM((D, S), BF),
            pltpu.VMEM((D, S), BF),
            pltpu.VMEM((S, A_QB), F32),
            pltpu.VMEM((S, A_QB), F32),
            pltpu.VMEM((1, A_QB), F32),
            pltpu.VMEM((1, A_QB), F32),
            pltpu.VMEM((64, A_QB), U32),
            pltpu.VMEM((D // 2, HD), U32),
            pltpu.VMEM((D // 2, HD), U32),
            pltpu.VMEM((D // 2, HD), U32),
            pltpu.VMEM((HD // 2, D), U32),
            pltpu.VMEM((n_seg * M, HD), BF),
            pltpu.VMEM((n_seg * M, HD), BF),
            pltpu.VMEM((n_seg * M, HD), BF),
            pltpu.VMEM((n_seg * M, HD), BF),
            pltpu.VMEM((S, D), F32),
            pltpu.VMEM((HB * (M + SEG), M + SEG), F32),
            pltpu.VMEM((D * HB, DHB), BF),
            pltpu.VMEM((D * HB, DHB), BF),
            pltpu.VMEM((D * HB, DHB), BF),
            pltpu.VMEM((HD, D), BF),
            pltpu.VMEM((D // 2, HB, DHB), U32),
            pltpu.VMEM((D // 2, HB, DHB), U32),
            pltpu.SemaphoreType.DMA((S // X_CH + 6,)),
        ],
        compiler_params=pltpu.CompilerParams(vmem_limit_bytes=120 * 1024 * 1024),
    )(A_x.reshape(S, D), A_wqkv, A_wo, B_mem0.reshape(M, D),
      B_Wq.reshape(D * HB, DHB), B_Wk.reshape(D * HB, DHB), B_Wv.reshape(D * HB, DHB),
      B_Wo.reshape(HD, D), gate_w.reshape(1, D))
    return out.reshape(B, S, D)
```

```python
import functools

import jax
import jax.numpy as jnp
from jax import lax
import jax.experimental.pallas as pl
import jax.experimental.pallas.tpu as pltpu

BF = jnp.bfloat16
F32 = jnp.float32
U32 = jnp.uint32
LOG2E = 1.4426950408889634
NEG_INF_SCORE = -1e9

A_QB = 512
A_KC = 256
B_PGW = 1024
B_WKC = 2
UNROLL = 2
X_CH = 512


def _branch_a(k_scr, qT_scr, vT_scr, oT_scr, sA, sB, mA, mB, qp, *, S, HA, DHA, QB, KC):
    HPG = 128 // DHA
    NQ = S // QB
    U = HA * NQ
    NC = S // KC

    def produce_setup(u):
        h = u // NQ
        qb = u % NQ
        g = h // HPG
        j = h % HPG
        goff = pl.multiple_of(g * 128, 128)
        qoff = pl.multiple_of(qb * QB, QB)
        RH = DHA // 2
        qh = qT_scr[pl.ds(pl.multiple_of(h * RH, RH), RH), pl.ds(qoff, QB)]
        rows = lax.broadcasted_iota(jnp.int32, (64, QB), 0)
        qp[...] = jnp.where((rows // RH) == j, jnp.concatenate([qh] * HPG, axis=0), jnp.uint32(0))
        return goff

    def step(up, uc, s_prod, m_prod, s_cons, m_cons):
        do_cons = s_cons is not None
        goff = produce_setup(up)
        if do_cons:
            hoff = pl.multiple_of((uc // NQ) * DHA, DHA)
            qoff = pl.multiple_of((uc % NQ) * QB, QB)
            ones_row = (lax.broadcasted_iota(jnp.int32, (DHA, S), 0) == 0).astype(BF)
            vTe = jnp.concatenate([vT_scr[pl.ds(hoff, DHA), :], ones_row], axis=0)
            mc = m_cons[...]
        mrun = None
        acc = None
        for c in range(NC):
            kc = pltpu.bitcast(k_scr[c * KC // 2:(c + 1) * KC // 2, pl.ds(goff, 128)], BF)
            s = jnp.dot(kc, pltpu.bitcast(qp[...], BF), preferred_element_type=F32)
            s_prod[c * KC:(c + 1) * KC, :] = s
            cm = jnp.max(s.reshape(KC // 8, 8, QB), axis=0)
            mrun = cm if mrun is None else jnp.maximum(mrun, cm)
            if do_cons:
                p = jnp.exp2(s_cons[c * KC:(c + 1) * KC, :] - mc).astype(BF)
                d = jnp.dot(vTe[:, c * KC:(c + 1) * KC], p, preferred_element_type=F32)
                acc = d if acc is None else acc + d
            if c < NC - 1:
                yield
        m_prod[...] = jnp.max(mrun, axis=0, keepdims=True)
        if do_cons:
            o = acc[0:DHA, :] / acc[DHA:DHA + 1, :]
            oT_scr[pl.ds(hoff, DHA), pl.ds(qoff, QB)] = o.astype(BF)
        yield

    def prologue():
        for _ in step(0, None, sA, mA, None, None):
            pass

    def gen(i):
        u0 = 2 * i
        yield from step(u0 + 1, u0, sB, mB, sA, mA)
        yield from step(jnp.minimum(u0 + 2, U - 1), u0 + 1, sA, mA, sB, mB)

    return prologue, gen


def _kernel(x_hbm, wqkv_hbm, woa_hbm, mem0_ref, wq_hbm, wk_hbm, wv_hbm, wob_hbm, gw_ref,
            out_hbm,
            x_ref, wqkv_ref, woa_ref, out_ref, osems,
            qT_scr, k_scr, vT_scr, oT_scr, sA, sB, mA, mB, qp,
            wq_p, wk_p, wv_p, wo_p, qpre, kpre, vpre, olate, b_scr, maskf,
            wq_raw, wk_raw, wv_raw, wo_raw, t0, t1, sems,
            *, S, D, HA, DHA, M, SEG, HB, DHB):
    NXC = S // X_CH
    x_copies = [pltpu.make_async_copy(x_hbm.at[pl.ds(c * X_CH, X_CH), :], x_ref.at[pl.ds(c * X_CH, X_CH), :],
                                      sems.at[c]) for c in range(NXC)]
    wqkv_copy = pltpu.make_async_copy(wqkv_hbm, wqkv_ref, sems.at[NXC])
    copies = [pltpu.make_async_copy(src, dst, sems.at[NXC + 1 + i]) for i, (src, dst) in enumerate(
        ((wq_hbm, wq_raw), (wk_hbm, wk_raw), (wv_hbm, wv_raw), (wob_hbm, wo_raw), (woa_hbm, woa_ref)))]
    wqkv_copy.start()
    for cp in x_copies + copies:
        cp.start()

    wqkv_copy.wait()
    for c in range(NXC):
        x_copies[c].wait()
        qkv = jnp.dot(x_ref[c * X_CH:(c + 1) * X_CH, :], wqkv_ref[...], preferred_element_type=F32)
        qT_scr[:, c * X_CH:(c + 1) * X_CH] = pltpu.bitcast(
            (qkv[:, 0:D] * (DHA ** -0.5 * LOG2E)).T.astype(BF), U32)
        k_scr[c * X_CH // 2:(c + 1) * X_CH // 2, :] = pltpu.bitcast(qkv[:, D:2 * D].astype(BF), U32)
        vT_scr[:, c * X_CH:(c + 1) * X_CH] = qkv[:, 2 * D:3 * D].T.astype(BF)
    a_prologue, a_gen = _branch_a(k_scr, qT_scr, vT_scr, oT_scr, sA, sB, mA, mB, qp,
                                  S=S, HA=HA, DHA=DHA, QB=A_QB, KC=A_KC)

    n_seg = S // SEG
    L = M + SEG
    NPRE = n_seg * M
    HD = HB * DHB
    HP = HB // 2
    cq = DHB ** -0.5 * LOG2E

    def wcols(ref, lo, hi):
        return pltpu.bitcast(ref[:, lo:hi], BF)

    def wrows(ref, lo, hi):
        return pltpu.bitcast(ref[lo // 2:hi // 2, :], BF)

    copies[0].wait()

    RP = D * HB // 2 // HP

    def step1_piece(raw, t, i):
        v = pltpu.bitcast(raw[2 * i * RP:2 * (i + 1) * RP, :], U32)
        t[i * RP // HB:(i + 1) * RP // HB, :, :] = v.reshape(RP // HB, HB, DHB)

    def unit(t, dst, hp):
        ev = t[:, hp, :]
        od = t[:, HP + hp, :]
        dst[:, (2 * hp) * DHB:(2 * hp + 1) * DHB] = (ev & jnp.uint32(0xFFFF)) | (od << 16)
        dst[:, (2 * hp + 1) * DHB:(2 * hp + 2) * DHB] = (ev >> 16) | (od & jnp.uint32(0xFFFF0000))

    WOP = HD // 2 // HP

    def wo_piece(i):
        wo_p[i * WOP:(i + 1) * WOP, :] = pltpu.bitcast(wo_raw[2 * i * WOP:2 * (i + 1) * WOP, :], U32)

    x_pre = x_ref[...].astype(F32).reshape(n_seg, SEG, D)[:, 0:M, :].reshape(NPRE, D).astype(BF)

    def prepass(w_p, pre, scl, hp):
        lo, hi = 2 * hp * DHB, (2 * hp + 2) * DHB
        y = jnp.dot(x_pre, wcols(w_p, lo, hi), preferred_element_type=F32)
        if scl is not None:
            y = y * scl
        pre[:, lo:hi] = y.astype(BF)

    for i in range(HP):
        step1_piece(wq_raw, t0, i)
    plan = ((wq_raw, t0, wq_p, qpre, cq), (wk_raw, t1, wk_p, kpre, None), (wv_raw, t0, wv_p, vpre, None))
    prev = None
    for mi, (raw, t, w_p, pre, scl) in enumerate(plan):
        copies[mi + 1].wait()
        for hp in range(HP):
            unit(t, w_p, hp)
            if mi + 1 < len(plan):
                step1_piece(plan[mi + 1][0], plan[mi + 1][1], hp)
            else:
                wo_piece(hp)
            if prev is not None:
                prepass(*prev)
            prev = (w_p, pre, scl, hp)
    prepass(*prev)

    ri = lax.broadcasted_iota(jnp.int32, (L, L), 0)
    ci = lax.broadcasted_iota(jnp.int32, (L, L), 1)
    tok_r = jnp.where(ri >= SEG, ri - SEG, ri)
    tok_c = jnp.where(ci >= SEG, ci - SEG, ci)
    mask = (ri < M) | (ci < M) | (tok_r >= tok_c)
    maskf[...] = jnp.concatenate([mask.astype(F32)] * HB, axis=0)

    a_prologue()

    NG = HD // B_PGW
    HPG = B_PGW // DHB
    HPW = HB // B_WKC

    def b_gen(s, mem, res):
        r0 = pl.multiple_of(s * SEG, SEG)
        p0 = pl.multiple_of(s * M, M)
        xs = x_ref[pl.ds(r0, SEG), :].astype(F32)
        hc = jnp.concatenate([mem, xs[M:SEG, :]], axis=0).astype(BF)
        qs, ks, vs = [], [], []
        for w_p, pre, lst, scl in ((wq_p, qpre, qs, cq), (wk_p, kpre, ks, None), (wv_p, vpre, vs, None)):
            for g in range(NG):
                lo, hi = g * B_PGW, (g + 1) * B_PGW
                y = jnp.dot(hc, wcols(w_p, lo, hi), preferred_element_type=F32)
                if scl is not None:
                    y = y * scl
                lst.append(jnp.concatenate([y.astype(BF), pre[pl.ds(p0, M), lo:hi]], axis=0))
                yield

        def head(lst, h):
            g, hh = divmod(h, HPG)
            return lst[g][:, hh * DHB:(hh + 1) * DHB]

        scs = []
        for h in range(HB):
            scs.append(lax.dot_general(head(qs, h), head(ks, h), (((1,), (1,)), ((), ())),
                                       preferred_element_type=F32))
            if h % 8 == 7:
                yield
        sc = jnp.concatenate(scs, axis=0)
        sc = jnp.where(maskf[...] > 0.5, sc, NEG_INF_SCORE * LOG2E)
        e = jnp.exp2(sc - jnp.max(sc, axis=-1, keepdims=True))
        l = jnp.sum(e, axis=-1, keepdims=True)
        r = pl.reciprocal(l, approx=True)
        p = e * (r * (2.0 - l * r))
        yield
        out32 = None
        lates = []
        for kc in range(B_WKC):
            outs = [jnp.dot(p[h * L:(h + 1) * L, :].astype(BF), head(vs, h), preferred_element_type=F32)
                    for h in range(kc * HPW, (kc + 1) * HPW)]
            o = jnp.concatenate(outs, axis=1)
            lates.append(o[SEG:L, :])
            yield
            d = jnp.dot(o[0:SEG, :].astype(BF), wrows(wo_p, kc * HPW * DHB, (kc + 1) * HPW * DHB),
                        preferred_element_type=F32)
            out32 = d if out32 is None else out32 + d
            yield
        olate[pl.ds(p0, M), :] = jnp.concatenate(lates, axis=1).astype(BF)
        b_scr[pl.ds(r0 + M, SEG - M), :] = out32[M:SEG, :]
        res.append(out32[0:M, :])

    def merged_body(s, mem):
        res = []
        ga, gb = a_gen(s), b_gen(s, mem, res)
        a_live = b_live = True
        while a_live or b_live:
            if a_live:
                a_live = next(ga, 'done') != 'done'
            if b_live:
                b_live = next(gb, 'done') != 'done'
        return res[0]

    lax.fori_loop(0, n_seg, merged_body, mem0_ref[...].astype(F32), unroll=UNROLL)

    copies[4].wait()
    SPC = X_CH // SEG
    out_copies = []
    for c in range(NXC):
        lo, hi = c * X_CH, (c + 1) * X_CH
        a = lax.dot_general(oT_scr[:, lo:hi], woa_ref[...], (((0,), (0,)), ((), ())),
                            preferred_element_type=F32)
        res = jnp.dot(olate[c * SPC * M:(c + 1) * SPC * M, :], wrows(wo_p, 0, HD),
                      preferred_element_type=F32)
        for s in range(SPC):
            b_scr[lo + s * SEG:lo + s * SEG + M, :] = res[s * M:(s + 1) * M, :]
        gl = jnp.sum(x_ref[lo:hi, :].astype(F32) * gw_ref[...].astype(F32), axis=-1, keepdims=True)
        g = jax.nn.sigmoid(gl)
        out_ref[lo:hi, :] = (g * a + (1.0 - g) * b_scr[lo:hi, :]).astype(out_ref.dtype)
        cp = pltpu.make_async_copy(out_ref.at[pl.ds(lo, X_CH), :], out_hbm.at[pl.ds(lo, X_CH), :], osems.at[c])
        cp.start()
        out_copies.append(cp)
    for cp in out_copies:
        cp.wait()


@functools.partial(jax.jit, static_argnames=("B_seg_len",))
def pallas_gated_mix__mha_block__memory_aug_recurrent_mem_tr__prompt_kernel(A_x, A_wqkv, A_wo, B_x, B_mem0, B_Wq, B_Wk, B_Wv, B_Wo, B_seg_len, gate_w):
    del B_x
    B, S, D = A_x.shape
    HA = 32
    DHA = D // HA
    Dm, HB, DHB = B_Wq.shape
    M = B_mem0.shape[1]
    SEG = int(B_seg_len)
    HD = HB * DHB
    n_seg = S // SEG
    assert S % X_CH == 0 and X_CH % SEG == 0
    assert B == 1 and Dm == D and S % SEG == 0 and S % A_QB == 0 and S % A_KC == 0
    assert 128 % DHA == 0 and DHA % 16 == 0 and DHB == 128 and HB % 2 == 0
    assert M % 8 == 0 and SEG % 16 == 0 and M < SEG and HD % B_PGW == 0 and HB % B_WKC == 0
    assert (HA * (S // A_QB)) % 2 == 0 and HA * (S // A_QB) // 2 == n_seg and n_seg % UNROLL == 0
    vmem = pl.BlockSpec(memory_space=pltpu.VMEM)
    hbm = pl.BlockSpec(memory_space=pl.ANY)
    kern = functools.partial(_kernel, S=S, D=D, HA=HA, DHA=DHA, M=M, SEG=SEG, HB=HB, DHB=DHB)
    out = pl.pallas_call(
        kern,
        out_shape=jax.ShapeDtypeStruct((S, D), A_x.dtype),
        in_specs=[hbm, hbm, hbm, vmem, hbm, hbm, hbm, hbm, vmem],
        out_specs=hbm,
        scratch_shapes=[
            pltpu.VMEM((S, D), BF),
            pltpu.VMEM((D, 3 * D), BF),
            pltpu.VMEM((D, D), BF),
            pltpu.VMEM((S, D), A_x.dtype),
            pltpu.SemaphoreType.DMA((S // X_CH,)),
            pltpu.VMEM((D // 2, S), U32),
            pltpu.VMEM((S // 2, D), U32),
            pltpu.VMEM((D, S), BF),
            pltpu.VMEM((D, S), BF),
            pltpu.VMEM((S, A_QB), F32),
            pltpu.VMEM((S, A_QB), F32),
            pltpu.VMEM((1, A_QB), F32),
            pltpu.VMEM((1, A_QB), F32),
            pltpu.VMEM((64, A_QB), U32),
            pltpu.VMEM((D // 2, HD), U32),
            pltpu.VMEM((D // 2, HD), U32),
            pltpu.VMEM((D // 2, HD), U32),
            pltpu.VMEM((HD // 2, D), U32),
            pltpu.VMEM((n_seg * M, HD), BF),
            pltpu.VMEM((n_seg * M, HD), BF),
            pltpu.VMEM((n_seg * M, HD), BF),
            pltpu.VMEM((n_seg * M, HD), BF),
            pltpu.VMEM((S, D), F32),
            pltpu.VMEM((HB * (M + SEG), M + SEG), F32),
            pltpu.VMEM((D * HB, DHB), BF),
            pltpu.VMEM((D * HB, DHB), BF),
            pltpu.VMEM((D * HB, DHB), BF),
            pltpu.VMEM((HD, D), BF),
            pltpu.VMEM((D // 2, HB, DHB), U32),
            pltpu.VMEM((D // 2, HB, DHB), U32),
            pltpu.SemaphoreType.DMA((S // X_CH + 6,)),
        ],
        compiler_params=pltpu.CompilerParams(vmem_limit_bytes=120 * 1024 * 1024),
    )(A_x.reshape(S, D), A_wqkv, A_wo, B_mem0.reshape(M, D),
      B_Wq.reshape(D * HB, DHB), B_Wk.reshape(D * HB, DHB), B_Wv.reshape(D * HB, DHB),
      B_Wo.reshape(HD, D), gate_w.reshape(1, D))
    return out.reshape(B, S, D)
```
